```python
import jax
import jax.numpy as jnp

def _softmax(x, axis=-1):
    return jax.nn.softmax(x, axis=axis)
def _gelu(x):
    return jax.nn.gelu(x, approximate=True)
def _silu(x):
    return jax.nn.silu(x)
def _sigmoid(x):
    return jax.nn.sigmoid(x)
def _layernorm(x, axis=-1, eps=1e-5):
    m = jnp.mean(x, axis=axis, keepdims=True)
    v = jnp.var(x, axis=axis, keepdims=True)
    return (x - m) / jnp.sqrt(v + eps)
def _scatter_add(tgt, idx, src, axis=0):
    return tgt.at[idx].add(src)
def _segment_sum(src, seg, n):
    return jax.ops.segment_sum(src, seg, n)
class _Rng:
    def __init__(self, key):
        self._k = key
    def _next(self):
        self._k, sub = jax.random.split(self._k)
        return sub
    def normal(self, shape):
        return jax.random.normal(self._next(), shape, dtype=jnp.bfloat16)
    def randint(self, lo, hi, shape):
        return jax.random.randint(self._next(), shape, lo, hi, dtype=jnp.int32)
    def uniform(self, shape, lo=0.0, hi=1.0):
        return jax.random.uniform(self._next(), shape, jnp.bfloat16, lo, hi)
    def permutation(self, n):
        return jax.random.permutation(self._next(), n)


kernel_name = 'sequential_preLN__sliding_block_cached__moe_arch_mod__decode'

def setup_inputs():
    _rng = _Rng(jax.random.key(int.from_bytes(__import__("os").urandom(4), "little")))
    _w = (lambda a: (lambda t: t.astype(jnp.bfloat16) if jnp.issubdtype(t.dtype, jnp.floating) else t)(jnp.asarray(a)))
    def _A_setup():
        B, Sq, D = 1, 1, 640
        Hq, Hkv, Sk, Dh = 32, 32, 32768, 192
        assert Hq % Hkv == 0, (Hq, Hkv)
        return {
            "x": _w((lambda *s: _rng.normal(s) * 0.05)(B, Sq, D)),
            "k_cache": _w((lambda *s: _rng.normal(s) * 0.05)(B, Hkv, Sk, Dh)),
            "v_cache": _w((lambda *s: _rng.normal(s) * 0.05)(B, Hkv, Sk, Dh)),
            "wq": _w((lambda *s: _rng.normal(s) * 0.05)(D, Hq * Dh) * (D ** -0.5)),
            "wo": _w((lambda *s: _rng.normal(s) * 0.05)(Hq * Dh, D) * ((Hq * Dh) ** -0.5)),
        }
    _A_in = _A_setup()

    def _B_setup():
        B, S, D, F, C = 1, 1, 640, 1536, 1
        return {
            "x": _w((lambda *s: _rng.normal(s) * 0.05)(B, S, D)),
            "w_r": _w((lambda *s: _rng.normal(s) * 0.05)(D)),
            "w_gate": _w((lambda *s: _rng.normal(s) * 0.05)(D, F)),
            "w_up": _w((lambda *s: _rng.normal(s) * 0.05)(D, F)),
            "w_down": _w((lambda *s: _rng.normal(s) * 0.05)(F, D)),
        }
    _B_in = _B_setup()

    return {
        "A_x": _A_in["x"],
        "A_k_cache": _A_in["k_cache"],
        "A_v_cache": _A_in["v_cache"],
        "A_wq": _A_in["wq"],
        "A_wo": _A_in["wo"],
        "B_x": _B_in["x"],
        "B_w_r": _B_in["w_r"],
        "B_w_gate": _B_in["w_gate"],
        "B_w_up": _B_in["w_up"],
        "B_w_down": _B_in["w_down"],
    }

def reference(A_x, A_k_cache, A_v_cache, A_wq, A_wo, B_x, B_w_r, B_w_gate, B_w_up, B_w_down):
    def _A_ref(x, k_cache, v_cache, wq, wo):
        B, Sq, D = x.shape
        Hq, Dh = 32, 192
        Hkv, Sk = k_cache.shape[1], k_cache.shape[2]
        W = min(4096, max(256, Sk // 4))
        rep = Hq // Hkv
        q = (lambda x, *d: x.transpose(*d))((x @ wq).reshape(B, Sq, Hq, Dh), 0, 2, 1, 3)
        k = jnp.repeat(k_cache[:, :, Sk - W:, :], rep, axis=1)
        v = jnp.repeat(v_cache[:, :, Sk - W:, :], rep, axis=1)
        scores = jnp.einsum("bhqd,bhkd->bhqk", q, k) * (Dh ** -0.5)
        p = _softmax(scores, axis=-1)
        o = jnp.einsum("bhqk,bhkd->bhqd", p, v)
        return (lambda x, *d: x.transpose(*d))(o, 0, 2, 1, 3).reshape(B, Sq, Hq * Dh) @ wo

    def _B_ref(x, w_r, w_gate, w_up, w_down):
        B, S, D = x.shape
        C = 1
        r = x @ w_r
        idx = jnp.argsort(-r, axis=-1)[:, :C]
        idx_e = jnp.repeat(idx.reshape(B, C, 1), D, axis=2)
        x_sel = jnp.take_along_axis(x, idx_e, axis=1)
        g = _silu(x_sel @ w_gate)
        u = x_sel @ w_up
        y = (g * u) @ w_down
        r_sel = _sigmoid(jnp.take_along_axis(r, idx, axis=1))
        y = y * r_sel.reshape(B, C, 1)
        b_off = (jnp.arange(B) * S).reshape(B, 1)
        flat_idx = (idx + b_off).reshape(B * C)
        zero = (x * 0.0).reshape(B * S, D)
        upd = _scatter_add(zero, flat_idx, y.reshape(B * C, D), axis=0)
        return x + upd.reshape(B, S, D)

    x = A_x
    h = x + _A_ref(_layernorm(x, axis=-1), A_k_cache, A_v_cache, A_wq, A_wo)
    h2 = h + _B_ref(_layernorm(h, axis=-1), B_w_r, B_w_gate, B_w_up, B_w_down)
    return h2
```

```python
import jax
import jax.numpy as jnp
from jax import lax
import jax.experimental.pallas as pl
import jax.experimental.pallas.tpu as pltpu

NBUF = 2
EPS = 1e-5


def _layernorm(x):
    m = jnp.mean(x, axis=-1, keepdims=True)
    d = x - m
    v = jnp.mean(d * d, axis=-1, keepdims=True)
    return d / jnp.sqrt(v + EPS)


def _kernel(x_hbm, kt_hbm, vt_hbm, wq_hbm, wo_hbm, wr_hbm, wg_hbm, wu_hbm, wd_hbm,
            o_ref,
            x_s, wr_s, wq_s, wo_s, wg_s, wu_s, wd_s, k_s, v_s, q_s, p_s, acc_s,
            sem_kv, sem_w, sem_d):
    _, H, Dh, Sk = kt_hbm.shape
    W = k_s.shape[-1]
    D = x_hbm.shape[-1]
    f32, bf16 = jnp.float32, jnp.bfloat16

    def done(dst, sem):
        pltpu.make_async_copy(dst, dst, sem).wait()

    def stream(trips, step, pieces, sem):
        def body(i, _):
            for n, (src, dst, r, nr, c, nc) in enumerate(pieces):
                idx = (pl.ds(pl.multiple_of(r + i * step, 8), nr), pl.ds(c, nc))
                pltpu.make_async_copy(src.at[idx], dst.at[idx], sem).start(priority=n % 2)
        lax.fori_loop(0, trips, body, None)

    def kv_start(h, slot):
        for c in range(0, W, 512):
            for r in range(0, Dh, 32):
                rows = pl.ds(r, 32)
                for prio, (src, dst) in enumerate(((kt_hbm, k_s), (vt_hbm, v_s))):
                    pltpu.make_async_copy(src.at[0, h, rows, pl.ds(Sk - W + c, 512)],
                                          dst.at[slot, rows, pl.ds(c, 512)],
                                          sem_kv.at[slot]).start(priority=prio)

    x_cp = pltpu.make_async_copy(x_hbm, x_s, sem_w.at[0])
    wr_cp = pltpu.make_async_copy(wr_hbm, wr_s, sem_w.at[0])
    x_cp.start()
    wr_cp.start(priority=1)
    stream(8, 8, [(wq_hbm, wq_s, s * 64, 8, c, 2048) for c in range(0, H * Dh, 2048) for s in range(10)],
           sem_w.at[0])
    stream(24, 32, [(wo_hbm, wo_s, s * 768, 32, 0, D) for s in range(8)], sem_w.at[0])
    kv_start(0, 0)
    x_cp.wait()
    wr_cp.wait()
    done(wq_s, sem_w.at[0])
    done(wo_s, sem_w.at[0])

    x = x_s[0].astype(f32)
    xn = jnp.broadcast_to(_layernorm(x), (8, D)).astype(bf16)
    QC = 2 * Dh
    for c in range(H // 2):
        q2 = jnp.dot(xn, wq_s[:, c * QC:(c + 1) * QC], preferred_element_type=f32)
        q_s[2 * c] = q2[:, :Dh]
        q_s[2 * c + 1] = q2[:, Dh:]
    acc_s[...] = jnp.zeros_like(acc_s)

    scale = Dh ** -0.5

    def head(h, _):
        slot = h % NBUF

        @pl.when(h + 1 < H)
        def _():
            kv_start(h + 1, (h + 1) % NBUF)

        @pl.when(h + 1 == H)
        def _():
            stream(8, 16, [(src, dst, s * 128, 16, 0, src.shape[1]) for s in range(5)
                           for src, dst in ((wg_hbm, wg_s), (wu_hbm, wu_s))], sem_w.at[1])

        done(k_s.at[slot], sem_kv.at[slot])
        done(v_s.at[slot], sem_kv.at[slot])
        s = jnp.dot(q_s[h].astype(bf16), k_s[slot], preferred_element_type=f32) * scale
        m = jnp.max(s, axis=-1, keepdims=True)
        e = jnp.exp(s - m)
        l = jnp.sum(e, axis=-1, keepdims=True)
        p_s[...] = e
        inv = 1.0 / l
        row0 = pl.multiple_of(h * Dh, 64)
        acc = acc_s[...]
        for r in range(Dh // 16):
            a0 = jnp.zeros((8, 128), f32)
            a1 = jnp.zeros((8, 128), f32)
            for j in range(W // 128):
                vv = v_s[slot, r * 16:(r + 1) * 16, j * 128:(j + 1) * 128].astype(f32)
                pp = p_s[:, j * 128:(j + 1) * 128]
                a0 = a0 + vv[:8] * pp
                a1 = a1 + vv[8:] * pp
            o0 = jnp.sum(a0, axis=-1, keepdims=True) * inv
            o1 = jnp.sum(a1, axis=-1, keepdims=True) * inv
            ww = wo_s[pl.ds(row0 + r * 16, 16), :].astype(f32)
            acc = acc + ww[:8] * o0 + ww[8:] * o1
        acc_s[...] = acc

    lax.fori_loop(0, H, head, None)

    down_chunks = ((0, 256), (256, 128))
    for c, (r0, nr) in enumerate(down_chunks):
        stream(nr // 32, 32, [(wd_hbm, wd_s, s * 384 + r0, 32, 0, D) for s in range(4)], sem_d.at[c])

    hres = x + jnp.sum(acc_s[...], axis=0, keepdims=True)
    hn = _layernorm(hres)
    wr = wr_s[...].astype(f32).reshape(1, D)
    gate = jax.nn.sigmoid(jnp.sum(hn * wr, axis=-1, keepdims=True))
    hb = jnp.broadcast_to(hn, (8, D)).astype(bf16)
    done(wg_s, sem_w.at[1])
    done(wu_s, sem_w.at[1])
    g = jnp.dot(hb, wg_s[...], preferred_element_type=f32)
    u = jnp.dot(hb, wu_s[...], preferred_element_type=f32)
    gu = (g * jax.nn.sigmoid(g) * u).astype(bf16)
    y = jnp.zeros((8, D), f32)
    for c, (r0, nr) in enumerate(down_chunks):
        for s in range(4):
            done(wd_s.at[pl.ds(s * 384 + r0, nr)], sem_d.at[c])
        for s in range(4):
            lo = s * 384 + r0
            y = y + jnp.dot(gu[:, lo:lo + nr], wd_s[lo:lo + nr, :], preferred_element_type=f32)
    out = hres + (hn + y[:1] * gate)
    o_ref[0] = out.astype(o_ref.dtype)


@jax.jit
def pallas_sequential_preLN__sliding_block_cached__moe_arch_mod__decode_kernel(
    A_x: jax.Array,
    A_k_cache: jax.Array,
    A_v_cache: jax.Array,
    A_wq: jax.Array,
    A_wo: jax.Array,
    B_x: jax.Array,
    B_w_r: jax.Array,
    B_w_gate: jax.Array,
    B_w_up: jax.Array,
    B_w_down: jax.Array,
):
    del B_x
    _, H, Sk, Dh = A_k_cache.shape
    D = A_x.shape[-1]
    W = min(4096, max(256, Sk // 4))
    kt = jnp.transpose(A_k_cache, (0, 1, 3, 2))
    vt = jnp.transpose(A_v_cache, (0, 1, 3, 2))
    like = lambda a: pltpu.VMEM(a.shape, a.dtype)
    return pl.pallas_call(
        _kernel,
        out_shape=jax.ShapeDtypeStruct(A_x.shape, A_x.dtype),
        in_specs=[pl.BlockSpec(memory_space=pl.ANY)] * 9,
        scratch_shapes=[
            like(A_x), like(B_w_r), like(A_wq), like(A_wo),
            like(B_w_gate), like(B_w_up), like(B_w_down),
            pltpu.VMEM((NBUF, Dh, W), A_k_cache.dtype),
            pltpu.VMEM((NBUF, Dh, W), A_v_cache.dtype),
            pltpu.VMEM((H, 8, Dh), jnp.float32),
            pltpu.VMEM((8, W), jnp.float32),
            pltpu.VMEM((8, D), jnp.float32),
            pltpu.SemaphoreType.DMA((NBUF,)), pltpu.SemaphoreType.DMA((2,)),
            pltpu.SemaphoreType.DMA((2,)),
        ],
        compiler_params=pltpu.CompilerParams(vmem_limit_bytes=100 * 2**20),
    )(A_x, kt, vt, A_wq, A_wo, B_w_r, B_w_gate, B_w_up, B_w_down)
```

```python
import jax
import jax.numpy as jnp
from jax import lax
import jax.experimental.pallas as pl
import jax.experimental.pallas.tpu as pltpu

EPS = 1e-5
BAND = 8
RUN = 512
LAG = 24
GROUPS_Q, GROUPS_O, GROUPS_F = 16, 12, 4
KV_ROWS = 96
DOWN_ROWS = 32
DOWN_CHUNKS = ((24, "mxu"), (36, "mxu"), (44, "vpu"), (47, "vpu"), (48, "vpu"))
SEM_ATTN, SEM_FFN, SEM_DOWN = 2, 3, 4


def _layernorm(x):
    m = jnp.mean(x, axis=-1, keepdims=True)
    d = x - m
    v = jnp.mean(d * d, axis=-1, keepdims=True)
    return d / jnp.sqrt(v + EPS)


def _kernel(x_hbm, kt_hbm, vt_hbm, wq_hbm, wo_hbm, wr_hbm, wg_hbm, wu_hbm, wd_hbm,
            o_ref,
            x_s, wr_s, wq_s, wo_s, wg_s, wu_s, wd_s, k_s, v_s, q_s, p_s, acc_s, sems):
    _, H, Dh, Sk = kt_hbm.shape
    W = k_s.shape[-1]
    D = x_hbm.shape[-1]
    F = wg_hbm.shape[-1]
    f32, bf16 = jnp.float32, jnp.bfloat16

    def copy(src, dst, sem, queue):
        pltpu.make_async_copy(src, dst, sems.at[sem]).start(priority=queue)

    def done(dst, sem):
        pltpu.make_async_copy(dst, dst, sems.at[sem]).wait()

    def piece(src, dst, group, groups, row, rows, col, cols, sem, queue):
        if not isinstance(row, int):
            row = pl.multiple_of(row, BAND)
        idx = (pl.ds(group, groups), pl.ds(row, rows), pl.ds(col, cols))
        copy(src.at[idx], dst.at[idx], sem, queue)

    def wq_band(row, lead=0):
        for n, (c, g) in enumerate((c, g) for c in range(0, H * Dh, RUN) for g in range(0, GROUPS_Q, 4)):
            piece(wq_hbm, wq_s, g, 4, row, BAND, c, RUN, SEM_ATTN, 1 if n < lead else n % 2)

    def wo_band(row):
        for n, g in enumerate(range(0, GROUPS_O, 3)):
            piece(wo_hbm, wo_s, g, 3, row, BAND, 0, D, SEM_ATTN, n % 2)

    def kv_start(h):
        slot = h % 2
        for blk in range(Dh // KV_ROWS):
            cols = range(0, W, RUN)
            for c in (reversed(cols) if blk % 2 else cols):
                for r in range(blk * KV_ROWS, (blk + 1) * KV_ROWS, 4 * BAND):
                    rows = pl.ds(r, 4 * BAND)
                    for queue, (src, dst) in enumerate(((kt_hbm, k_s), (vt_hbm, v_s))):
                        copy(src.at[0, h, rows, pl.ds(Sk - W + c, RUN)],
                             dst.at[slot, rows, pl.ds(c, RUN)], slot, queue)

    ffn_band = [(src, dst, c) for c in range(0, F, RUN) for src, dst in ((wg_hbm, wg_s), (wu_hbm, wu_s))]
    ffn_bands = wg_s.shape[1] // BAND
    late_bands = LAG // len(ffn_band)

    def ffn_start():
        def body(i, _):
            for n, (src, dst, c) in enumerate(ffn_band):
                piece(src, dst, 0, GROUPS_F, i * BAND, BAND, c, RUN, SEM_FFN, n % 2)
        lax.fori_loop(0, ffn_bands - late_bands, body, None)

    def down_piece(j, queue):
        chunk = next(i for i, (end, _) in enumerate(DOWN_CHUNKS) if j < end)
        piece(wd_hbm, wd_s, j % GROUPS_F, 1, j // GROUPS_F * DOWN_ROWS, DOWN_ROWS, 0, D,
              SEM_DOWN + chunk, queue)

    def tail_start():
        pairs = (DOWN_CHUNKS[-1][0] - LAG) // 2
        early = [2 * i + 1 for i in range(pairs)] + list(range(2 * pairs, pairs + LAG))
        late = [(b, *band) for b in range(ffn_bands - late_bands, ffn_bands) for band in ffn_band]
        for (b, src, dst, c), j in zip(late, early, strict=True):
            piece(src, dst, 0, GROUPS_F, b * BAND, BAND, c, RUN, SEM_FFN, 0)
            down_piece(j, 1)
        for i in range(pairs):
            down_piece(2 * i, 0)
            down_piece(pairs + LAG + i, 1)

    def matvec(v, w_s, c0, nc):
        w = w_s[:, :, c0:c0 + nc]
        return jnp.dot(v, w.reshape(-1, nc), preferred_element_type=f32)

    x_cp = pltpu.make_async_copy(x_hbm, x_s, sems.at[SEM_ATTN])
    wr_cp = pltpu.make_async_copy(wr_hbm, wr_s, sems.at[SEM_ATTN])
    wq_band(0, lead=LAG + 2)
    x_cp.start()
    wr_cp.start()
    lax.fori_loop(1, wq_s.shape[1] // BAND, lambda i, _: wq_band(i * BAND), None)
    lax.fori_loop(0, wo_s.shape[1] // BAND, lambda i, _: wo_band(i * BAND), None)

    def project_q():
        x_cp.wait()
        wr_cp.wait()
        done(wq_s, SEM_ATTN)
        done(wo_s, SEM_ATTN)
        xn = jnp.broadcast_to(_layernorm(x_s[0].astype(f32)), (8, D)).astype(bf16)
        for c in range(H // 2):
            q2 = matvec(xn, wq_s, c * 2 * Dh, 2 * Dh)
            q_s[2 * c] = q2[:, :Dh]
            q_s[2 * c + 1] = q2[:, Dh:]
        acc_s[...] = jnp.zeros_like(acc_s)

    def attend(h):
        slot = h % 2
        done(k_s.at[slot], slot)
        done(v_s.at[slot], slot)
        s = jnp.dot(q_s[h].astype(bf16), k_s[slot], preferred_element_type=f32) * Dh ** -0.5
        m = jnp.max(s, axis=-1, keepdims=True)
        e = jnp.exp(s - m)
        inv = 1.0 / jnp.sum(e, axis=-1, keepdims=True)
        p_s[...] = e
        acc = acc_s[...]
        for r in range(0, Dh, 16):
            a0 = jnp.zeros((8, 128), f32)
            a1 = jnp.zeros((8, 128), f32)
            for c in range(0, W, 128):
                vv = v_s[slot, r:r + 16, c:c + 128].astype(f32)
                pp = p_s[:, c:c + 128]
                a0 = a0 + vv[:8] * pp
                a1 = a1 + vv[8:] * pp
            o0 = jnp.sum(a0, axis=-1, keepdims=True) * inv
            o1 = jnp.sum(a1, axis=-1, keepdims=True) * inv
            row = h * Dh + r
            sub = pl.multiple_of(lax.rem(row, wo_s.shape[1]), 16)
            ww = wo_s[lax.div(row, wo_s.shape[1]), pl.ds(sub, 16), :].astype(f32)
            acc = acc + ww[:8] * o0 + ww[8:] * o1
        acc_s[...] = acc

    def step(i, _):
        pl.when(i < H)(lambda: kv_start(i))
        pl.when(i == H)(ffn_start)
        pl.when(i == 0)(project_q)
        pl.when(i > 0)(lambda: attend(i - 1))

    lax.fori_loop(0, H + 1, step, None)
    tail_start()

    hres = x_s[0].astype(f32) + jnp.sum(acc_s[...], axis=0, keepdims=True)
    hn = _layernorm(hres)
    wr = wr_s[...].astype(f32).reshape(1, D)
    gate = jax.nn.sigmoid(jnp.sum(hn * wr, axis=-1, keepdims=True))
    hb = jnp.broadcast_to(hn, (8, D)).astype(bf16)
    done(wg_s, SEM_FFN)
    done(wu_s, SEM_FFN)
    g = matvec(hb, wg_s, 0, F)
    act = g * jax.nn.sigmoid(g) * matvec(hb, wu_s, 0, F)
    act_b = act.astype(bf16)

    group_rows = wd_s.shape[1]
    chunks, start = [], 0
    for end, unit in DOWN_CHUNKS:
        spans = []
        for grp in range(GROUPS_F):
            js = [j for j in range(start, end) if j % GROUPS_F == grp]
            if js:
                spans.append((grp, js[0] // GROUPS_F * DOWN_ROWS, len(js) * DOWN_ROWS))
        chunks.append((unit, spans))
        start = end
    act_t = {}
    for unit, spans in chunks:
        for grp, r0, nr in spans if unit == "vpu" else ():
            for row in range(grp * group_rows + r0, grp * group_rows + r0 + nr, BAND):
                t = row // 128 * 128
                if t not in act_t:
                    act_t[t] = jnp.broadcast_to(act[:1, t:t + 128] * gate, (128, 128)).T

    y = jnp.zeros((8, D), f32)
    out = None
    for c, (unit, spans) in enumerate(chunks):
        for grp, r0, nr in spans:
            done(wd_s.at[grp, pl.ds(r0, nr)], SEM_DOWN + c)
        if unit == "mxu":
            for grp, r0, nr in spans:
                row = grp * group_rows + r0
                y = y + jnp.dot(act_b[:, row:row + nr], wd_s[grp, r0:r0 + nr, :],
                                preferred_element_type=f32)
            continue
        if out is None:
            first = lax.broadcasted_iota(jnp.int32, (8, D), 0) == 0
            out = jnp.where(first, jnp.broadcast_to(hres + hn + y[:1] * gate, (8, D)), 0.0)
        for grp, r0, nr in spans:
            for r in range(r0, r0 + nr, BAND):
                row = grp * group_rows + r
                a = act_t[row // 128 * 128][row % 128:row % 128 + BAND]
                out = out + wd_s[grp, r:r + BAND, :].astype(f32) * jnp.concatenate([a] * (D // 128), axis=1)
    for c in range(0, D, 128):
        o_ref[0, :, c:c + 128] = jnp.sum(out[:, c:c + 128], axis=0, keepdims=True).astype(o_ref.dtype)


@jax.jit
def pallas_sequential_preLN__sliding_block_cached__moe_arch_mod__decode_kernel(
    A_x: jax.Array,
    A_k_cache: jax.Array,
    A_v_cache: jax.Array,
    A_wq: jax.Array,
    A_wo: jax.Array,
    B_x: jax.Array,
    B_w_r: jax.Array,
    B_w_gate: jax.Array,
    B_w_up: jax.Array,
    B_w_down: jax.Array,
):
    del B_x
    _, H, Sk, Dh = A_k_cache.shape
    D = A_x.shape[-1]
    W = min(4096, max(256, Sk // 4))
    kt = jnp.transpose(A_k_cache, (0, 1, 3, 2))
    vt = jnp.transpose(A_v_cache, (0, 1, 3, 2))
    grouped = lambda w, groups: w.reshape(groups, w.shape[0] // groups, w.shape[1])
    wq, wo = grouped(A_wq, GROUPS_Q), grouped(A_wo, GROUPS_O)
    wg, wu, wd = (grouped(w, GROUPS_F) for w in (B_w_gate, B_w_up, B_w_down))
    like = lambda a: pltpu.VMEM(a.shape, a.dtype)
    return pl.pallas_call(
        _kernel,
        out_shape=jax.ShapeDtypeStruct(A_x.shape, A_x.dtype),
        in_specs=[pl.BlockSpec(memory_space=pl.ANY)] * 9,
        scratch_shapes=[
            like(A_x), like(B_w_r), like(wq), like(wo), like(wg), like(wu), like(wd),
            pltpu.VMEM((2, Dh, W), A_k_cache.dtype),
            pltpu.VMEM((2, Dh, W), A_v_cache.dtype),
            pltpu.VMEM((H, 8, Dh), jnp.float32),
            pltpu.VMEM((8, W), jnp.float32),
            pltpu.VMEM((8, D), jnp.float32),
            pltpu.SemaphoreType.DMA((SEM_DOWN + len(DOWN_CHUNKS),)),
        ],
        compiler_params=pltpu.CompilerParams(
            vmem_limit_bytes=100 * 2**20,
            disable_bounds_checks=True,
            disable_semaphore_checks=True,
        ),
    )(A_x, kt, vt, wq, wo, B_w_r, wg, wu, wd)
```

```python
import jax
import jax.numpy as jnp
from jax import lax
import jax.experimental.pallas as pl
import jax.experimental.pallas.tpu as pltpu

EPS = 1e-5
BAND = 8
RUN = 512
LAG = 24
SLAB = 128
GROUPS_F = 4
KV_ROWS = 96
SLOTS = 3
Q_PARTS = 4
DOWN_ROWS = 32
DOWN_CHUNKS = ((24, "mxu"), (36, "mxu"), (44, "vpu"), (47, "vpu"), (48, "vpu"))
SEM_ATTN, SEM_FFN, SEM_DOWN = SLOTS, SLOTS + 1, SLOTS + 2


def _layernorm(x):
    m = jnp.mean(x, axis=-1, keepdims=True)
    d = x - m
    v = jnp.mean(d * d, axis=-1, keepdims=True)
    return d / jnp.sqrt(v + EPS)


def _kernel(x_hbm, kt_hbm, vt_hbm, wq_hbm, wo_hbm, wr_hbm, wg_hbm, wu_hbm, wd_hbm,
            o_ref,
            x_s, wr_s, wq_s, wo_s, wg_s, wu_s, wd_s, k_s, v_s, xt_s, q_s, p_s, acc_s, sems):
    _, H, Dh, Sk = kt_hbm.shape
    W = k_s.shape[-1]
    D = x_hbm.shape[-1]
    F = wg_hbm.shape[-1]
    f32, bf16 = jnp.float32, jnp.bfloat16

    def copy(src, dst, sem, queue):
        pltpu.make_async_copy(src, dst, sems.at[sem]).start(priority=queue)

    def done(dst, sem):
        pltpu.make_async_copy(dst, dst, sems.at[sem]).wait()

    def piece(src, dst, group, groups, row, rows, col, cols, sem, queue):
        if not isinstance(row, int):
            row = pl.multiple_of(row, BAND)
        idx = (pl.ds(group, groups), pl.ds(row, rows), pl.ds(col, cols))
        copy(src.at[idx], dst.at[idx], sem, queue)

    sweep_pieces = [(g, src, dst) for g in range(0, wq_s.shape[0], 3)
                    for src, dst in ((wq_hbm, wq_s), (wo_hbm, wo_s))]

    def attn_sweep(i, lead=0):
        for n, (g, src, dst) in enumerate(sweep_pieces):
            idx = (pl.ds(g, 3), pl.ds(2 * i, 2))
            copy(src.at[idx], dst.at[idx], SEM_ATTN, 1 if n < lead else n % 2)

    def kv_start(h):
        slot = h % SLOTS
        for blk in range(Dh // KV_ROWS):
            cols = range(0, W, RUN)
            for c in (reversed(cols) if blk % 2 else cols):
                for r in range(blk * KV_ROWS, (blk + 1) * KV_ROWS, 4 * BAND):
                    rows = pl.ds(r, 4 * BAND)
                    for queue, (src, dst) in enumerate(((kt_hbm, k_s), (vt_hbm, v_s))):
                        copy(src.at[0, h, rows, pl.ds(Sk - W + c, RUN)],
                             dst.at[slot, rows, pl.ds(c, RUN)], slot, queue)

    ffn_band = [(src, dst, c) for c in range(0, F, RUN) for src, dst in ((wg_hbm, wg_s), (wu_hbm, wu_s))]
    ffn_bands = wg_s.shape[1] // BAND
    late_bands = LAG // len(ffn_band)

    def ffn_start():
        def body(i, _):
            for n, (src, dst, c) in enumerate(ffn_band):
                piece(src, dst, 0, GROUPS_F, i * BAND, BAND, c, RUN, SEM_FFN, n % 2)
        lax.fori_loop(0, ffn_bands - late_bands, body, None)

    def down_piece(j, queue):
        chunk = next(i for i, (end, _) in enumerate(DOWN_CHUNKS) if j < end)
        piece(wd_hbm, wd_s, j % GROUPS_F, 1, j // GROUPS_F * DOWN_ROWS, DOWN_ROWS, 0, D,
              SEM_DOWN + chunk, queue)

    def tail_start():
        pairs = (DOWN_CHUNKS[-1][0] - LAG) // 2
        early = [2 * i + 1 for i in range(pairs)] + list(range(2 * pairs, pairs + LAG))
        late = [(b, *band) for b in range(ffn_bands - late_bands, ffn_bands) for band in ffn_band]
        for (b, src, dst, c), j in zip(late, early, strict=True):
            piece(src, dst, 0, GROUPS_F, b * BAND, BAND, c, RUN, SEM_FFN, 0)
            down_piece(j, 1)
        for i in range(pairs):
            down_piece(2 * i, 0)
            down_piece(pairs + LAG + i, 1)

    def matvec(v, w_s):
        w = w_s[...]
        return jnp.dot(v, w.reshape(-1, w.shape[-1]), preferred_element_type=f32)

    x_cp = pltpu.make_async_copy(x_hbm, x_s, sems.at[SEM_ATTN])
    wr_cp = pltpu.make_async_copy(wr_hbm, wr_s, sems.at[SEM_ATTN])
    lead = LAG + 4
    peeled = pl.cdiv(lead, len(sweep_pieces))
    for i in range(peeled):
        attn_sweep(i, lead - i * len(sweep_pieces))
    x_cp.start()
    wr_cp.start()
    lax.fori_loop(peeled, SLAB // 2, lambda i, _: attn_sweep(i), None)

    def normalize_x():
        x_cp.wait()
        wr_cp.wait()
        done(wq_s, SEM_ATTN)
        done(wo_s, SEM_ATTN)
        xn = _layernorm(x_s[0].astype(f32)).astype(bf16).astype(f32)
        for c in range(0, D, 128):
            xt_s[c:c + 128, :] = jnp.broadcast_to(xn[:, c:c + 128], (128, 128)).T
        acc_s[...] = jnp.zeros_like(acc_s)

    def project_q(part):
        band_pairs = H * Dh // 256
        quads = H // 4 // Q_PARTS
        for c in range(part * quads, (part + 1) * quads):
            a = [jnp.zeros((8, 128), f32)] * 6
            for b in range(D // BAND):
                xb = xt_s[b * BAND:(b + 1) * BAND, :]
                for j in range(3):
                    m = b * band_pairs + 3 * c + j
                    ww = wq_s[m // SLAB, m % SLAB].astype(f32)
                    a[2 * j] = a[2 * j] + ww[:8] * xb
                    a[2 * j + 1] = a[2 * j + 1] + ww[8:] * xb
            q4 = jnp.concatenate(
                [jnp.broadcast_to(jnp.sum(t, axis=0, keepdims=True), (8, 128)) for t in a], axis=1)
            for k in range(4):
                q_s[4 * c + k] = q4[:, k * Dh:(k + 1) * Dh]

    def attend(h):
        slot = h % SLOTS
        done(k_s.at[slot], slot)
        done(v_s.at[slot], slot)
        s = jnp.dot(q_s[h].astype(bf16), k_s[slot], preferred_element_type=f32) * Dh ** -0.5
        m = jnp.max(s, axis=-1, keepdims=True)
        e = jnp.exp(s - m)
        inv = 1.0 / jnp.sum(e, axis=-1, keepdims=True)
        p_s[...] = e
        tiles = D // 128
        acc = [acc_s[:, t * 128:(t + 1) * 128] for t in range(tiles)]
        for r in range(0, Dh, 16):
            a0 = jnp.zeros((8, 128), f32)
            a1 = jnp.zeros((8, 128), f32)
            for c in range(0, W, 128):
                vv = v_s[slot, r:r + 16, c:c + 128].astype(f32)
                pp = p_s[:, c:c + 128]
                a0 = a0 + vv[:8] * pp
                a1 = a1 + vv[8:] * pp
            o0 = jnp.sum(a0, axis=-1, keepdims=True) * inv
            o1 = jnp.sum(a1, axis=-1, keepdims=True) * inv
            for j in range(tiles):
                m = h * (Dh // 16 * tiles) + r // 16 * tiles + j
                ww = wo_s[lax.div(m, SLAB), lax.rem(m, SLAB)].astype(f32)
                for n, w in ((2 * j, ww[:8]), (2 * j + 1, ww[8:])):
                    acc[n % tiles] = acc[n % tiles] + w * (o0 if n < tiles else o1)
        for t in range(tiles):
            acc_s[:, t * 128:(t + 1) * 128] = acc[t]

    def step(i, _):
        pl.when(i < H)(lambda: kv_start(i))
        pl.when(i == H)(ffn_start)
        pl.when(i == H + 1)(tail_start)
        pl.when(i == 1)(normalize_x)
        for part in range(Q_PARTS):
            pl.when(i == 1 + part)(lambda part=part: project_q(part))
        pl.when(i >= SLOTS - 1)(lambda: attend(i - (SLOTS - 1)))

    lax.fori_loop(0, H + SLOTS - 1, step, None)

    hres = x_s[0].astype(f32) + jnp.sum(acc_s[...], axis=0, keepdims=True)
    hn = _layernorm(hres)
    wr = wr_s[...].astype(f32).reshape(1, D)
    gate = jax.nn.sigmoid(jnp.sum(hn * wr, axis=-1, keepdims=True))
    hb = jnp.broadcast_to(hn, (8, D)).astype(bf16)
    done(wg_s, SEM_FFN)
    done(wu_s, SEM_FFN)
    g = matvec(hb, wg_s)
    act = g * jax.nn.sigmoid(g) * matvec(hb, wu_s)
    act_b = act.astype(bf16)

    group_rows = wd_s.shape[1]
    chunks, start = [], 0
    for end, unit in DOWN_CHUNKS:
        spans = []
        for grp in range(GROUPS_F):
            js = [j for j in range(start, end) if j % GROUPS_F == grp]
            if js:
                spans.append((grp, js[0] // GROUPS_F * DOWN_ROWS, len(js) * DOWN_ROWS))
        chunks.append((unit, spans))
        start = end
    act_t = {}
    for unit, spans in chunks:
        for grp, r0, nr in spans if unit == "vpu" else ():
            for row in range(grp * group_rows + r0, grp * group_rows + r0 + nr, BAND):
                t = row // 128 * 128
                if t not in act_t:
                    act_t[t] = jnp.broadcast_to(act[:1, t:t + 128] * gate, (128, 128)).T

    y = jnp.zeros((8, D), f32)
    out = None
    for c, (unit, spans) in enumerate(chunks):
        for grp, r0, nr in spans:
            done(wd_s.at[grp, pl.ds(r0, nr)], SEM_DOWN + c)
        if unit == "mxu":
            for grp, r0, nr in spans:
                row = grp * group_rows + r0
                y = y + jnp.dot(act_b[:, row:row + nr], wd_s[grp, r0:r0 + nr, :],
                                preferred_element_type=f32)
            continue
        if out is None:
            first = lax.broadcasted_iota(jnp.int32, (8, D), 0) == 0
            out = jnp.where(first, jnp.broadcast_to(hres + hn + y[:1] * gate, (8, D)), 0.0)
        for grp, r0, nr in spans:
            for r in range(r0, r0 + nr, BAND):
                row = grp * group_rows + r
                a = act_t[row // 128 * 128][row % 128:row % 128 + BAND]
                out = out + wd_s[grp, r:r + BAND, :].astype(f32) * jnp.concatenate([a] * (D // 128), axis=1)
    for c in range(0, D, 128):
        o_ref[0, :, c:c + 128] = jnp.sum(out[:, c:c + 128], axis=0, keepdims=True).astype(o_ref.dtype)


@jax.jit
def pallas_sequential_preLN__sliding_block_cached__moe_arch_mod__decode_kernel(
    A_x: jax.Array,
    A_k_cache: jax.Array,
    A_v_cache: jax.Array,
    A_wq: jax.Array,
    A_wo: jax.Array,
    B_x: jax.Array,
    B_w_r: jax.Array,
    B_w_gate: jax.Array,
    B_w_up: jax.Array,
    B_w_down: jax.Array,
):
    del B_x
    _, H, Sk, Dh = A_k_cache.shape
    D = A_x.shape[-1]
    W = min(4096, max(256, Sk // 4))
    kt = jnp.transpose(A_k_cache, (0, 1, 3, 2))
    vt = jnp.transpose(A_v_cache, (0, 1, 3, 2))

    def tile_pairs(w):
        t = w.reshape(w.shape[0] // BAND, BAND, w.shape[1] // 128, 128).transpose(0, 2, 1, 3)
        return t.reshape(-1, SLAB, 2 * BAND, 128)

    wq, wo = tile_pairs(A_wq), tile_pairs(A_wo)
    wg, wu, wd = (w.reshape(GROUPS_F, -1, w.shape[1]) for w in (B_w_gate, B_w_up, B_w_down))
    like = lambda a: pltpu.VMEM(a.shape, a.dtype)
    return pl.pallas_call(
        _kernel,
        out_shape=jax.ShapeDtypeStruct(A_x.shape, A_x.dtype),
        in_specs=[pl.BlockSpec(memory_space=pl.ANY)] * 9,
        scratch_shapes=[
            like(A_x), like(B_w_r), like(wq), like(wo), like(wg), like(wu), like(wd),
            pltpu.VMEM((SLOTS, Dh, W), A_k_cache.dtype),
            pltpu.VMEM((SLOTS, Dh, W), A_v_cache.dtype),
            pltpu.VMEM((D, 128), jnp.float32),
            pltpu.VMEM((H, 8, Dh), jnp.float32),
            pltpu.VMEM((8, W), jnp.float32),
            pltpu.VMEM((8, D), jnp.float32),
            pltpu.SemaphoreType.DMA((SEM_DOWN + len(DOWN_CHUNKS),)),
        ],
        compiler_params=pltpu.CompilerParams(
            vmem_limit_bytes=100 * 2**20,
            disable_bounds_checks=True,
            disable_semaphore_checks=True,
        ),
    )(A_x, kt, vt, wq, wo, B_w_r, wg, wu, wd)
```

```python
import jax
import jax.numpy as jnp
from jax import lax
import jax.experimental.pallas as pl
import jax.experimental.pallas.tpu as pltpu

EPS = 1e-5
BAND = 8
RUN = 512
SLAB = 128
LAG = 28
ATTN_RUNS, KV_RUNS = 3, 4
GROUPS_F = 4
DOWN_ROWS = 32
SLOTS = 4
Q_PARTS = 4
DOWN_CHUNKS = ((24, "mxu"), (36, "mxu"), (44, "vpu"), (47, "vpu"), (48, "vpu"))
SEM_ATTN, SEM_FFN, SEM_DOWN = SLOTS, SLOTS + 1, SLOTS + 2


def _layernorm(x):
    m = jnp.mean(x, axis=-1, keepdims=True)
    d = x - m
    v = jnp.mean(d * d, axis=-1, keepdims=True)
    return d / jnp.sqrt(v + EPS)


def _kernel(x_hbm, kt_hbm, vt_hbm, wq_hbm, wo_hbm, wr_hbm, wg_hbm, wu_hbm, wd_hbm,
            o_ref,
            x_s, wr_s, wq_s, wo_s, wg_s, wu_s, wd_s, k_s, v_s, xt_s, q_s, p_s, acc_s, sems):
    _, H, Dh, Sk = kt_hbm.shape
    W = k_s.shape[-1]
    D = x_hbm.shape[-1]
    F = wg_hbm.shape[-1]
    f32, bf16 = jnp.float32, jnp.bfloat16

    def start(piece, queue):
        src, dst, sem = piece
        pltpu.make_async_copy(src, dst, sems.at[sem]).start(priority=queue)

    def start_pairs(first, second):
        for a, b in zip(first, second, strict=True):
            start(a, 0)
            start(b, 1)

    def done(dst, sem):
        pltpu.make_async_copy(dst, dst, sems.at[sem]).wait()

    per_sweep = wq_s.shape[0] // ATTN_RUNS

    def attn_piece(src, dst, sweep, n):
        idx = (pl.ds(n % per_sweep * ATTN_RUNS, ATTN_RUNS), pl.ds(2 * (sweep + n // per_sweep), 2))
        return src.at[idx], dst.at[idx], SEM_ATTN

    def kv_pieces(h, half):
        slot = h % SLOTS
        return [(src.at[0, h, pl.ds(r, KV_RUNS * BAND), pl.ds(Sk - W + c, RUN)],
                 dst.at[slot, pl.ds(r, KV_RUNS * BAND), pl.ds(c, RUN)], slot)
                for src, dst in ((kt_hbm, k_s), (vt_hbm, v_s))
                for c in range(0, W, RUN)
                for r in range(half * Dh // 2, (half + 1) * Dh // 2, KV_RUNS * BAND)]

    def ffn_pieces(src, dst):
        return [(src.at[:, pl.ds(r, BAND), pl.ds(c, RUN)], dst.at[:, pl.ds(r, BAND), pl.ds(c, RUN)], SEM_FFN)
                for r in range(0, dst.shape[1], BAND) for c in range(0, F, RUN)]

    def down_piece(j):
        chunk = next(i for i, (end, _) in enumerate(DOWN_CHUNKS) if j < end)
        idx = (j % GROUPS_F, pl.ds(j // GROUPS_F * DOWN_ROWS, DOWN_ROWS))
        return wd_hbm.at[idx], wd_s.at[idx], SEM_DOWN + chunk

    def start_tail(third):
        count = DOWN_CHUNKS[-1][0]
        pairs = (count - LAG) // 2
        first = ffn_pieces(wg_hbm, wg_s) + [down_piece(2 * i) for i in range(pairs)]
        second = (ffn_pieces(wu_hbm, wu_s)[LAG:] + [down_piece(2 * i + 1) for i in range(pairs)]
                  + [down_piece(j) for j in range(2 * pairs, count)])
        lo, hi = third * len(first) // 3, (third + 1) * len(first) // 3
        start_pairs(first[lo:hi], second[lo:hi])

    x_cp = pltpu.make_async_copy(x_hbm, x_s, sems.at[SEM_ATTN])
    wr_cp = pltpu.make_async_copy(wr_hbm, wr_s, sems.at[SEM_ATTN])
    for n in range(LAG):
        start(attn_piece(wo_hbm, wo_s, 0, n), 1)
    x_cp.start()
    wr_cp.start()

    def sweep(i, _):
        start_pairs([attn_piece(wq_hbm, wq_s, i, n) for n in range(per_sweep)],
                    [attn_piece(wo_hbm, wo_s, i, LAG + n) for n in range(per_sweep)])

    total = SLAB // 2 * per_sweep
    looped = (total - LAG) // per_sweep
    lax.fori_loop(0, looped, sweep, None)
    start_pairs([attn_piece(wq_hbm, wq_s, 0, n) for n in range(looped * per_sweep, total)],
                [attn_piece(wo_hbm, wo_s, 0, n) for n in range(looped * per_sweep + LAG, total)]
                + kv_pieces(0, 1)[:LAG])

    def normalize_x():
        x_cp.wait()
        wr_cp.wait()
        done(wq_s, SEM_ATTN)
        done(wo_s, SEM_ATTN)
        xn = _layernorm(x_s[0].astype(f32)).astype(bf16).astype(f32)
        for c in range(0, D, 128):
            xt_s[c:c + 128, :] = jnp.broadcast_to(xn[:, c:c + 128], (128, 128)).T
        acc_s[...] = jnp.zeros_like(acc_s)

    def project_q(part):
        band_pairs = H * Dh // 256
        quads = H // 4 // Q_PARTS
        for c in range(part * quads, (part + 1) * quads):
            a = [jnp.zeros((8, 128), f32)] * 6
            for b in range(D // BAND):
                xb = xt_s[b * BAND:(b + 1) * BAND, :]
                for j in range(3):
                    m = b * band_pairs + 3 * c + j
                    ww = wq_s[m // SLAB, m % SLAB].astype(f32)
                    a[2 * j] = a[2 * j] + ww[:8] * xb
                    a[2 * j + 1] = a[2 * j + 1] + ww[8:] * xb
            q4 = jnp.concatenate(
                [jnp.broadcast_to(jnp.sum(t, axis=0, keepdims=True), (8, 128)) for t in a], axis=1)
            for k in range(4):
                q_s[4 * c + k] = q4[:, k * Dh:(k + 1) * Dh]

    def probabilities(h):
        slot = h % SLOTS
        done(k_s.at[slot], slot)
        done(v_s.at[slot], slot)
        s = jnp.dot(q_s[h].astype(bf16), k_s[slot], preferred_element_type=f32) * Dh ** -0.5
        e = jnp.exp(s - jnp.max(s, axis=-1, keepdims=True))
        p_s[...] = e * (1.0 / jnp.sum(e, axis=-1, keepdims=True))

    def accumulate(h):
        slot = h % SLOTS
        tiles = D // 128
        acc = [acc_s[:, t * 128:(t + 1) * 128] for t in range(tiles)]
        for r in range(0, Dh, 16):
            a0 = jnp.zeros((8, 128), f32)
            a1 = jnp.zeros((8, 128), f32)
            for c in range(0, W, 128):
                vv = v_s[slot, r:r + 16, c:c + 128].astype(f32)
                pp = p_s[:, c:c + 128]
                a0 = a0 + vv[:8] * pp
                a1 = a1 + vv[8:] * pp
            o0 = jnp.sum(a0, axis=-1, keepdims=True)
            o1 = jnp.sum(a1, axis=-1, keepdims=True)
            for j in range(tiles):
                m = h * (Dh // 16 * tiles) + r // 16 * tiles + j
                ww = wo_s[lax.div(m, SLAB), lax.rem(m, SLAB)].astype(f32)
                for n, w in ((2 * j, ww[:8]), (2 * j + 1, ww[8:])):
                    acc[n % tiles] = acc[n % tiles] + w * (o0 if n < tiles else o1)
        for t in range(tiles):
            acc_s[:, t * 128:(t + 1) * 128] = acc[t]

    def step(i, _):
        cut = Dh // (KV_RUNS * BAND) * (W // RUN) - LAG
        pl.when(i < H)(lambda: start_pairs(kv_pieces(i, 0)[:cut], kv_pieces(i, 1)[LAG:]))
        pl.when(i == H)(lambda: start_tail(0))
        pl.when(i == 1)(normalize_x)
        for part in range(Q_PARTS):
            pl.when(i == 1 + part)(lambda part=part: project_q(part))
        pl.when(i >= 2)(lambda: probabilities(i - 2))
        pl.when(i < H - 1)(lambda: start_pairs(kv_pieces(i, 0)[cut:], kv_pieces(i + 1, 1)[:LAG]))
        pl.when(i == H - 1)(
            lambda: start_pairs(kv_pieces(H - 1, 0)[cut:], ffn_pieces(wu_hbm, wu_s)[:LAG]))
        pl.when(i == H)(lambda: start_tail(1))
        pl.when(i == H + 1)(lambda: start_tail(2))
        pl.when(i >= 2)(lambda: accumulate(i - 2))

    lax.fori_loop(0, H + 2, step, None)

    def matvec(v, w_s):
        w = w_s[...]
        return jnp.dot(v, w.reshape(-1, w.shape[-1]), preferred_element_type=f32)

    hres = x_s[0].astype(f32) + jnp.sum(acc_s[...], axis=0, keepdims=True)
    hn = _layernorm(hres)
    wr = wr_s[...].astype(f32).reshape(1, D)
    gate = jax.nn.sigmoid(jnp.sum(hn * wr, axis=-1, keepdims=True))
    hb = jnp.broadcast_to(hn, (8, D)).astype(bf16)
    done(wg_s, SEM_FFN)
    done(wu_s, SEM_FFN)
    g = matvec(hb, wg_s)
    act = g * jax.nn.sigmoid(g) * matvec(hb, wu_s)
    act_b = act.astype(bf16)

    group_rows = wd_s.shape[1]
    chunks, lo = [], 0
    for end, unit in DOWN_CHUNKS:
        spans = []
        for grp in range(GROUPS_F):
            js = [j for j in range(lo, end) if j % GROUPS_F == grp]
            if js:
                spans.append((grp, js[0] // GROUPS_F * DOWN_ROWS, len(js) * DOWN_ROWS))
        chunks.append((unit, spans))
        lo = end
    act_t = {}
    for unit, spans in chunks:
        for grp, r0, nr in spans if unit == "vpu" else ():
            for row in range(grp * group_rows + r0, grp * group_rows + r0 + nr, BAND):
                t = row // 128 * 128
                if t not in act_t:
                    act_t[t] = jnp.broadcast_to(act[:1, t:t + 128] * gate, (128, 128)).T

    y = jnp.zeros((8, D), f32)
    out = None
    for c, (unit, spans) in enumerate(chunks):
        for grp, r0, nr in spans:
            done(wd_s.at[grp, pl.ds(r0, nr)], SEM_DOWN + c)
        if unit == "mxu":
            for grp, r0, nr in spans:
                row = grp * group_rows + r0
                y = y + jnp.dot(act_b[:, row:row + nr], wd_s[grp, r0:r0 + nr, :],
                                preferred_element_type=f32)
            continue
        if out is None:
            first = lax.broadcasted_iota(jnp.int32, (8, D), 0) == 0
            out = jnp.where(first, jnp.broadcast_to(hres + hn + y[:1] * gate, (8, D)), 0.0)
        for grp, r0, nr in spans:
            for r in range(r0, r0 + nr, BAND):
                row = grp * group_rows + r
                a = act_t[row // 128 * 128][row % 128:row % 128 + BAND]
                out = out + wd_s[grp, r:r + BAND, :].astype(f32) * jnp.concatenate([a] * (D // 128), axis=1)
    for c in range(0, D, 128):
        o_ref[0, :, c:c + 128] = jnp.sum(out[:, c:c + 128], axis=0, keepdims=True).astype(o_ref.dtype)


@jax.jit
def pallas_sequential_preLN__sliding_block_cached__moe_arch_mod__decode_kernel(
    A_x: jax.Array,
    A_k_cache: jax.Array,
    A_v_cache: jax.Array,
    A_wq: jax.Array,
    A_wo: jax.Array,
    B_x: jax.Array,
    B_w_r: jax.Array,
    B_w_gate: jax.Array,
    B_w_up: jax.Array,
    B_w_down: jax.Array,
):
    del B_x
    _, H, Sk, Dh = A_k_cache.shape
    D = A_x.shape[-1]
    W = min(4096, max(256, Sk // 4))
    kt = jnp.transpose(A_k_cache, (0, 1, 3, 2))
    vt = jnp.transpose(A_v_cache, (0, 1, 3, 2))

    def tile_pairs(w):
        t = w.reshape(w.shape[0] // BAND, BAND, w.shape[1] // 128, 128).transpose(0, 2, 1, 3)
        return t.reshape(-1, SLAB, 2 * BAND, 128)

    wq, wo = tile_pairs(A_wq), tile_pairs(A_wo)
    wg, wu, wd = (w.reshape(GROUPS_F, -1, w.shape[1]) for w in (B_w_gate, B_w_up, B_w_down))
    like = lambda a: pltpu.VMEM(a.shape, a.dtype)
    return pl.pallas_call(
        _kernel,
        out_shape=jax.ShapeDtypeStruct(A_x.shape, A_x.dtype),
        in_specs=[pl.BlockSpec(memory_space=pl.ANY)] * 9,
        scratch_shapes=[
            like(A_x), like(B_w_r), like(wq), like(wo), like(wg), like(wu), like(wd),
            pltpu.VMEM((SLOTS, Dh, W), A_k_cache.dtype),
            pltpu.VMEM((SLOTS, Dh, W), A_v_cache.dtype),
            pltpu.VMEM((D, 128), jnp.float32),
            pltpu.VMEM((H, 8, Dh), jnp.float32),
            pltpu.VMEM((8, W), jnp.float32),
            pltpu.VMEM((8, D), jnp.float32),
            pltpu.SemaphoreType.DMA((SEM_DOWN + len(DOWN_CHUNKS),)),
        ],
        compiler_params=pltpu.CompilerParams(
            vmem_limit_bytes=100 * 2**20,
            disable_semaphore_checks=True,
        ),
    )(A_x, kt, vt, wq, wo, B_w_r, wg, wu, wd)
```

```python
import jax
import jax.numpy as jnp
from jax import lax
import jax.experimental.pallas as pl
import jax.experimental.pallas.tpu as pltpu

EPS = 1e-5
BAND = 8
RUN = 512
SLAB = 128
LAG = 27
ATTN_RUNS, KV_RUNS = 3, 4
GROUPS_F = 4
DOWN_ROWS = 32
SLOTS = 4
Q_PARTS = 4
DOWN_CHUNKS = ((24, "mxu"), (36, "mxu"), (44, "vpu"), (45, "vpu"), (46, "vpu"), (47, "vpu"), (48, "vpu"))
SEM_K, SEM_V = 0, SLOTS
SEM_X, SEM_R, SEM_Q, SEM_O, SEM_GATE, SEM_UP, SEM_DOWN = range(2 * SLOTS, 2 * SLOTS + 7)


def _layernorm(x):
    m = jnp.mean(x, axis=-1, keepdims=True)
    d = x - m
    v = jnp.mean(d * d, axis=-1, keepdims=True)
    return d / jnp.sqrt(v + EPS)


def _kernel(x_hbm, kt_hbm, vt_hbm, wq_hbm, wo_hbm, wr_hbm, wg_hbm, wu_hbm, wd_hbm,
            o_ref,
            x_s, wr_s, wq_s, wo_s, wg_s, wu_s, wd_s, k_s, v_s, xt_s, q_s, p_s, acc_s, sems):
    _, H, Dh, Sk = kt_hbm.shape
    W = k_s.shape[-1]
    D = x_hbm.shape[-1]
    F = wg_hbm.shape[-1]
    f32, bf16 = jnp.float32, jnp.bfloat16

    def start(piece, queue):
        src, dst, sem = piece
        pltpu.make_async_copy(src, dst, sems.at[sem]).start(priority=queue)

    def start_pairs(first, second):
        for a, b in zip(first, second, strict=True):
            start(a, 0)
            start(b, 1)

    def done(dst, sem):
        pltpu.make_async_copy(dst, dst, sems.at[sem]).wait()

    per_sweep = wq_s.shape[0] // ATTN_RUNS

    wq, wo = (wq_hbm, wq_s, SEM_Q), (wo_hbm, wo_s, SEM_O)
    wg, wu = (wg_hbm, wg_s, SEM_GATE), (wu_hbm, wu_s, SEM_UP)

    def attn_piece(weight, sweep, n):
        src, dst, sem = weight
        idx = (pl.ds(n % per_sweep * ATTN_RUNS, ATTN_RUNS), pl.ds(2 * (sweep + n // per_sweep), 2))
        return src.at[idx], dst.at[idx], sem

    def kv_pieces(h, half):
        slot = h % SLOTS
        return [(src.at[0, h, pl.ds(r, KV_RUNS * BAND), pl.ds(Sk - W + c, RUN)],
                 dst.at[slot, pl.ds(r, KV_RUNS * BAND), pl.ds(c, RUN)], sem + slot)
                for src, dst, sem in ((kt_hbm, k_s, SEM_K), (vt_hbm, v_s, SEM_V))
                for c in range(0, W, RUN)
                for r in range(half * Dh // 2, (half + 1) * Dh // 2, KV_RUNS * BAND)]

    def ffn_pieces(weight):
        src, dst, sem = weight
        return [(src.at[:, pl.ds(r, BAND), pl.ds(c, RUN)], dst.at[:, pl.ds(r, BAND), pl.ds(c, RUN)], sem)
                for r in range(0, dst.shape[1], BAND) for c in range(0, F, RUN)]

    def down_piece(j):
        chunk = next(i for i, (end, _) in enumerate(DOWN_CHUNKS) if j < end)
        idx = (j % GROUPS_F, pl.ds(j // GROUPS_F * DOWN_ROWS, DOWN_ROWS))
        return wd_hbm.at[idx], wd_s.at[idx], SEM_DOWN + chunk

    def start_tail(third):
        count = DOWN_CHUNKS[-1][0]
        pairs = (count - LAG) // 2
        first = ffn_pieces(wg) + [down_piece(2 * i) for i in range(pairs)]
        second = (ffn_pieces(wu)[LAG:] + [down_piece(2 * i + 1) for i in range(pairs)]
                  + [down_piece(j) for j in range(2 * pairs, count)])
        lo, hi = third * len(first) // 3, (third + 1) * len(first) // 3
        start_pairs(first[lo:hi], second[lo:hi])
        if third == 2:
            for piece in second[hi:]:
                start(piece, 1)

    x_cp = pltpu.make_async_copy(x_hbm, x_s, sems.at[SEM_X])
    wr_cp = pltpu.make_async_copy(wr_hbm, wr_s, sems.at[SEM_R])
    for n in range(LAG):
        start(attn_piece(wo, 0, n), 1)
    x_cp.start()
    wr_cp.start()

    def sweep(i, _):
        start_pairs([attn_piece(wq, i, n) for n in range(per_sweep)],
                    [attn_piece(wo, i, LAG + n) for n in range(per_sweep)])

    total = SLAB // 2 * per_sweep
    looped = (total - LAG) // per_sweep
    lax.fori_loop(0, looped, sweep, None)
    start_pairs([attn_piece(wq, 0, n) for n in range(looped * per_sweep, total)],
                [attn_piece(wo, 0, n) for n in range(looped * per_sweep + LAG, total)]
                + kv_pieces(0, 1)[:LAG])

    def normalize_x():
        x_cp.wait()
        wr_cp.wait()
        done(wq_s, SEM_Q)
        done(wo_s, SEM_O)
        xn = _layernorm(x_s[0].astype(f32)).astype(bf16).astype(f32)
        for c in range(0, D, 128):
            xt_s[c:c + 128, :] = jnp.broadcast_to(xn[:, c:c + 128], (128, 128)).T
        acc_s[...] = jnp.zeros_like(acc_s)

    def project_q(part):
        band_pairs = H * Dh // 256
        quads = H // 4 // Q_PARTS
        for c in range(part * quads, (part + 1) * quads):
            a = [jnp.zeros((8, 128), f32)] * 6
            for b in range(D // BAND):
                xb = xt_s[b * BAND:(b + 1) * BAND, :]
                for j in range(3):
                    m = b * band_pairs + 3 * c + j
                    ww = wq_s[m // SLAB, m % SLAB].astype(f32)
                    a[2 * j] = a[2 * j] + ww[:8] * xb
                    a[2 * j + 1] = a[2 * j + 1] + ww[8:] * xb
            q4 = jnp.concatenate(
                [jnp.broadcast_to(jnp.sum(t, axis=0, keepdims=True), (8, 128)) for t in a], axis=1)
            for k in range(4):
                q_s[4 * c + k] = q4[:, k * Dh:(k + 1) * Dh]

    def probabilities(h):
        slot = h % SLOTS
        done(k_s.at[slot], SEM_K + slot)
        s = jnp.dot(q_s[h].astype(bf16), k_s[slot], preferred_element_type=f32) * Dh ** -0.5
        e = jnp.exp(s - jnp.max(s, axis=-1, keepdims=True))
        p_s[...] = e * (1.0 / jnp.sum(e, axis=-1, keepdims=True))

    def accumulate(h):
        slot = h % SLOTS
        done(v_s.at[slot], SEM_V + slot)
        tiles = D // 128
        acc = [acc_s[:, t * 128:(t + 1) * 128] for t in range(tiles)]
        for r in range(0, Dh, 16):
            a0 = jnp.zeros((8, 128), f32)
            a1 = jnp.zeros((8, 128), f32)
            for c in range(0, W, 128):
                vv = v_s[slot, r:r + 16, c:c + 128].astype(f32)
                pp = p_s[:, c:c + 128]
                a0 = a0 + vv[:8] * pp
                a1 = a1 + vv[8:] * pp
            o0 = jnp.sum(a0, axis=-1, keepdims=True)
            o1 = jnp.sum(a1, axis=-1, keepdims=True)
            for j in range(tiles):
                m = h * (Dh // 16 * tiles) + r // 16 * tiles + j
                ww = wo_s[lax.div(m, SLAB), lax.rem(m, SLAB)].astype(f32)
                for n, w in ((2 * j, ww[:8]), (2 * j + 1, ww[8:])):
                    acc[n % tiles] = acc[n % tiles] + w * (o0 if n < tiles else o1)
        for t in range(tiles):
            acc_s[:, t * 128:(t + 1) * 128] = acc[t]

    def step(i, _):
        cut = Dh // (KV_RUNS * BAND) * (W // RUN) - LAG
        pl.when(i < H)(lambda: start_pairs(kv_pieces(i, 0)[:cut], kv_pieces(i, 1)[LAG:]))
        pl.when(i == H)(lambda: start_tail(0))
        pl.when(i == 1)(normalize_x)
        for part in range(Q_PARTS):
            pl.when(i == 1 + part)(lambda part=part: project_q(part))
        pl.when(i >= 2)(lambda: probabilities(i - 2))
        pl.when(i < H - 1)(lambda: start_pairs(kv_pieces(i, 0)[cut:], kv_pieces(i + 1, 1)[:LAG]))
        pl.when(i == H - 1)(lambda: start_pairs(kv_pieces(H - 1, 0)[cut:], ffn_pieces(wu)[:LAG]))
        pl.when(i == H)(lambda: start_tail(1))
        pl.when(i == H + 1)(lambda: start_tail(2))
        pl.when(i >= 2)(lambda: accumulate(i - 2))

    lax.fori_loop(0, H + 2, step, None)

    def matvec(v, w_s):
        w = w_s[...]
        return jnp.dot(v, w.reshape(-1, w.shape[-1]), preferred_element_type=f32)

    hres = x_s[0].astype(f32) + jnp.sum(acc_s[...], axis=0, keepdims=True)
    hn = _layernorm(hres)
    wr = wr_s[...].astype(f32).reshape(1, D)
    gate = jax.nn.sigmoid(jnp.sum(hn * wr, axis=-1, keepdims=True))
    hb = jnp.broadcast_to(hn, (8, D)).astype(bf16)
    done(wg_s, SEM_GATE)
    done(wu_s, SEM_UP)
    g = matvec(hb, wg_s)
    act = g * jax.nn.sigmoid(g) * matvec(hb, wu_s)
    act_b = act.astype(bf16)

    group_rows = wd_s.shape[1]
    chunks, lo = [], 0
    for end, unit in DOWN_CHUNKS:
        groups = range(GROUPS_F) if end - lo > 1 else (lo % GROUPS_F,)
        chunks.append((unit, groups, lo // GROUPS_F * DOWN_ROWS, (end - lo) // len(groups) * DOWN_ROWS))
        lo = end
    act_t = {}
    for unit, groups, r0, nr in chunks:
        for grp in groups if unit == "vpu" else ():
            for row in range(grp * group_rows + r0, grp * group_rows + r0 + nr, BAND):
                t = row // 128 * 128
                if t not in act_t:
                    act_t[t] = jnp.broadcast_to(act[:1, t:t + 128] * gate, (128, 128)).T

    y = jnp.zeros((8, D), f32)
    out = None
    for c, (unit, groups, r0, nr) in enumerate(chunks):
        done(wd_s.at[pl.ds(groups[0], len(groups)), pl.ds(r0, nr)], SEM_DOWN + c)
        if unit == "mxu":
            for grp in groups:
                row = grp * group_rows + r0
                y = y + jnp.dot(act_b[:, row:row + nr], wd_s[grp, r0:r0 + nr, :],
                                preferred_element_type=f32)
            continue
        if out is None:
            first = lax.broadcasted_iota(jnp.int32, (8, D), 0) == 0
            out = jnp.where(first, jnp.broadcast_to(hres + hn + y[:1] * gate, (8, D)), 0.0)
        for grp in groups:
            for r in range(r0, r0 + nr, BAND):
                row = grp * group_rows + r
                a = act_t[row // 128 * 128][row % 128:row % 128 + BAND]
                out = out + wd_s[grp, r:r + BAND, :].astype(f32) * jnp.concatenate([a] * (D // 128), axis=1)
    for c in range(0, D, 128):
        o_ref[0, :, c:c + 128] = jnp.sum(out[:, c:c + 128], axis=0, keepdims=True).astype(o_ref.dtype)


@jax.jit
def pallas_sequential_preLN__sliding_block_cached__moe_arch_mod__decode_kernel(
    A_x: jax.Array,
    A_k_cache: jax.Array,
    A_v_cache: jax.Array,
    A_wq: jax.Array,
    A_wo: jax.Array,
    B_x: jax.Array,
    B_w_r: jax.Array,
    B_w_gate: jax.Array,
    B_w_up: jax.Array,
    B_w_down: jax.Array,
):
    del B_x
    _, H, Sk, Dh = A_k_cache.shape
    D = A_x.shape[-1]
    W = min(4096, max(256, Sk // 4))
    kt = jnp.transpose(A_k_cache, (0, 1, 3, 2))
    vt = jnp.transpose(A_v_cache, (0, 1, 3, 2))

    def tile_pairs(w):
        t = w.reshape(w.shape[0] // BAND, BAND, w.shape[1] // 128, 128).transpose(0, 2, 1, 3)
        return t.reshape(-1, SLAB, 2 * BAND, 128)

    wq, wo = tile_pairs(A_wq), tile_pairs(A_wo)
    wg, wu, wd = (w.reshape(GROUPS_F, -1, w.shape[1]) for w in (B_w_gate, B_w_up, B_w_down))
    like = lambda a: pltpu.VMEM(a.shape, a.dtype)
    return pl.pallas_call(
        _kernel,
        out_shape=jax.ShapeDtypeStruct(A_x.shape, A_x.dtype),
        in_specs=[pl.BlockSpec(memory_space=pl.ANY)] * 9,
        scratch_shapes=[
            like(A_x), like(B_w_r), like(wq), like(wo), like(wg), like(wu), like(wd),
            pltpu.VMEM((SLOTS, Dh, W), A_k_cache.dtype),
            pltpu.VMEM((SLOTS, Dh, W), A_v_cache.dtype),
            pltpu.VMEM((D, 128), jnp.float32),
            pltpu.VMEM((H, 8, Dh), jnp.float32),
            pltpu.VMEM((8, W), jnp.float32),
            pltpu.VMEM((8, D), jnp.float32),
            pltpu.SemaphoreType.DMA((SEM_DOWN + len(DOWN_CHUNKS),)),
        ],
        compiler_params=pltpu.CompilerParams(
            vmem_limit_bytes=100 * 2**20,
            disable_semaphore_checks=True,
        ),
    )(A_x, kt, vt, wq, wo, B_w_r, wg, wu, wd)
```

```python
import jax
import jax.numpy as jnp
from jax import lax
import jax.experimental.pallas as pl
import jax.experimental.pallas.tpu as pltpu

EPS = 1e-5
BAND = 8
RUN = 512
SLAB = 128
LAG = 27
ATTN_RUNS, KV_RUNS = 3, 4
GROUPS_F = 4
SLOTS = 4
Q_PARTS = 4
DOWN_CHUNKS = (
    ("mxu", range(0, 4), 0, 128, 32), ("mxu", range(0, 4), 128, 128, 32),
    ("vpu", range(0, 3), 256, 64, 32), ("vpu", range(0, 3), 320, 64, 32),
    ("vpu", range(3, 4), 256, 40, 40), ("vpu", range(3, 4), 296, 40, 40),
    ("vpu", range(3, 4), 336, 32, 32), ("vpu", range(3, 4), 368, 16, 16),
)
SEM_K, SEM_V = 0, SLOTS
SEM_X, SEM_R, SEM_Q, SEM_O, SEM_GATE, SEM_UP, SEM_DOWN = range(2 * SLOTS, 2 * SLOTS + 7)


def _layernorm(x):
    m = jnp.mean(x, axis=-1, keepdims=True)
    d = x - m
    v = jnp.mean(d * d, axis=-1, keepdims=True)
    return d / jnp.sqrt(v + EPS)


def _kernel(x_hbm, kt_hbm, vt_hbm, wq_hbm, wo_hbm, wr_hbm, wg_hbm, wu_hbm, wd_hbm,
            o_ref,
            x_s, wr_s, wq_s, wo_s, wg_s, wu_s, wd_s, k_s, v_s, xt_s, q_s, p_s, acc_s, sems):
    _, H, Dh, Sk = kt_hbm.shape
    W = k_s.shape[-1]
    D = x_hbm.shape[-1]
    F = wg_hbm.shape[-1]
    f32, bf16 = jnp.float32, jnp.bfloat16

    def start(piece, queue):
        src, dst, sem = piece
        pltpu.make_async_copy(src, dst, sems.at[sem]).start(priority=queue)

    def start_pairs(first, second):
        for a, b in zip(first, second, strict=True):
            start(a, 0)
            start(b, 1)

    def done(dst, sem):
        pltpu.make_async_copy(dst, dst, sems.at[sem]).wait()

    per_sweep = wq_s.shape[0] // ATTN_RUNS

    wq, wo = (wq_hbm, wq_s, SEM_Q), (wo_hbm, wo_s, SEM_O)
    wg, wu = (wg_hbm, wg_s, SEM_GATE), (wu_hbm, wu_s, SEM_UP)

    def attn_piece(weight, sweep, n):
        src, dst, sem = weight
        idx = (pl.ds(n % per_sweep * ATTN_RUNS, ATTN_RUNS), pl.ds(2 * (sweep + n // per_sweep), 2))
        return src.at[idx], dst.at[idx], sem

    def kv_pieces(h, half):
        slot = h % SLOTS
        return [(src.at[0, h, pl.ds(r, KV_RUNS * BAND), pl.ds(Sk - W + c, RUN)],
                 dst.at[slot, pl.ds(r, KV_RUNS * BAND), pl.ds(c, RUN)], sem + slot)
                for src, dst, sem in ((kt_hbm, k_s, SEM_K), (vt_hbm, v_s, SEM_V))
                for c in range(0, W, RUN)
                for r in range(half * Dh // 2, (half + 1) * Dh // 2, KV_RUNS * BAND)]

    def ffn_pieces(weight):
        src, dst, sem = weight
        return [(src.at[:, pl.ds(r, BAND), pl.ds(c, RUN)], dst.at[:, pl.ds(r, BAND), pl.ds(c, RUN)], sem)
                for r in range(0, dst.shape[1], BAND) for c in range(0, F, RUN)]

    def start_tail(third):
        down = [(wd_hbm.at[grp, pl.ds(r, step)], wd_s.at[grp, pl.ds(r, step)], SEM_DOWN + c)
                for c, (_, groups, r0, rows, step) in enumerate(DOWN_CHUNKS)
                for r in range(r0, r0 + rows, step) for grp in groups]
        paired = (len(down) - LAG) // 2 * 2
        first = ffn_pieces(wg) + down[0:paired:2]
        second = ffn_pieces(wu)[LAG:] + down[1:paired:2] + down[paired:]
        lo, hi = third * len(first) // 3, (third + 1) * len(first) // 3
        start_pairs(first[lo:hi], second[lo:hi])
        if third == 2:
            for piece in second[hi:]:
                start(piece, 1)

    x_cp = pltpu.make_async_copy(x_hbm, x_s, sems.at[SEM_X])
    wr_cp = pltpu.make_async_copy(wr_hbm, wr_s, sems.at[SEM_R])
    for n in range(LAG):
        start(attn_piece(wo, 0, n), 1)
    x_cp.start()
    wr_cp.start()

    def sweep(i, _):
        start_pairs([attn_piece(wq, i, n) for n in range(per_sweep)],
                    [attn_piece(wo, i, LAG + n) for n in range(per_sweep)])

    total = SLAB // 2 * per_sweep
    looped = (total - LAG) // per_sweep
    lax.fori_loop(0, looped, sweep, None)
    start_pairs([attn_piece(wq, 0, n) for n in range(looped * per_sweep, total)],
                [attn_piece(wo, 0, n) for n in range(looped * per_sweep + LAG, total)]
                + kv_pieces(0, 1)[:LAG])

    def normalize_x():
        x_cp.wait()
        wr_cp.wait()
        done(wq_s, SEM_Q)
        done(wo_s, SEM_O)
        xn = _layernorm(x_s[0].astype(f32)).astype(bf16).astype(f32)
        for c in range(0, D, 128):
            xt_s[c:c + 128, :] = jnp.broadcast_to(xn[:, c:c + 128], (128, 128)).T
        acc_s[...] = jnp.zeros_like(acc_s)

    def project_q(part):
        band_pairs = H * Dh // 256
        quads = H // 4 // Q_PARTS
        for c in range(part * quads, (part + 1) * quads):
            a = [jnp.zeros((8, 128), f32)] * 6
            for b in range(D // BAND):
                xb = xt_s[b * BAND:(b + 1) * BAND, :]
                for j in range(3):
                    m = b * band_pairs + 3 * c + j
                    ww = wq_s[m // SLAB, m % SLAB].astype(f32)
                    a[2 * j] = a[2 * j] + ww[:8] * xb
                    a[2 * j + 1] = a[2 * j + 1] + ww[8:] * xb
            q4 = jnp.concatenate(
                [jnp.broadcast_to(jnp.sum(t, axis=0, keepdims=True), (8, 128)) for t in a], axis=1)
            for k in range(4):
                q_s[4 * c + k] = q4[:, k * Dh:(k + 1) * Dh]

    def probabilities(h):
        slot = h % SLOTS
        done(k_s.at[slot], SEM_K + slot)
        s = jnp.dot(q_s[h].astype(bf16), k_s[slot], preferred_element_type=f32) * Dh ** -0.5
        e = jnp.exp(s - jnp.max(s, axis=-1, keepdims=True))
        p_s[...] = e * (1.0 / jnp.sum(e, axis=-1, keepdims=True))

    def accumulate(h):
        slot = h % SLOTS
        done(v_s.at[slot], SEM_V + slot)
        tiles = D // 128
        acc = [acc_s[:, t * 128:(t + 1) * 128] for t in range(tiles)]
        for r in range(0, Dh, 16):
            a0 = jnp.zeros((8, 128), f32)
            a1 = jnp.zeros((8, 128), f32)
            for c in range(0, W, 128):
                vv = v_s[slot, r:r + 16, c:c + 128].astype(f32)
                pp = p_s[:, c:c + 128]
                a0 = a0 + vv[:8] * pp
                a1 = a1 + vv[8:] * pp
            o0 = jnp.sum(a0, axis=-1, keepdims=True)
            o1 = jnp.sum(a1, axis=-1, keepdims=True)
            for j in range(tiles):
                m = h * (Dh // 16 * tiles) + r // 16 * tiles + j
                ww = wo_s[lax.div(m, SLAB), lax.rem(m, SLAB)].astype(f32)
                for n, w in ((2 * j, ww[:8]), (2 * j + 1, ww[8:])):
                    acc[n % tiles] = acc[n % tiles] + w * (o0 if n < tiles else o1)
        for t in range(tiles):
            acc_s[:, t * 128:(t + 1) * 128] = acc[t]

    def step(i, _):
        cut = Dh // (KV_RUNS * BAND) * (W // RUN) - LAG
        pl.when(i < H)(lambda: start_pairs(kv_pieces(i, 0)[:cut], kv_pieces(i, 1)[LAG:]))
        pl.when(i == H)(lambda: start_tail(0))
        pl.when(i == 1)(normalize_x)
        for part in range(Q_PARTS):
            pl.when(i == 1 + part)(lambda part=part: project_q(part))
        pl.when(i >= 2)(lambda: probabilities(i - 2))
        pl.when(i < H - 1)(lambda: start_pairs(kv_pieces(i, 0)[cut:], kv_pieces(i + 1, 1)[:LAG]))
        pl.when(i == H - 1)(lambda: start_pairs(kv_pieces(H - 1, 0)[cut:], ffn_pieces(wu)[:LAG]))
        pl.when(i == H)(lambda: start_tail(1))
        pl.when(i == H + 1)(lambda: start_tail(2))
        pl.when(i >= 2)(lambda: accumulate(i - 2))

    lax.fori_loop(0, H + 2, step, None)

    def matvec(v, w_s):
        w = w_s[...]
        return jnp.dot(v, w.reshape(-1, w.shape[-1]), preferred_element_type=f32)

    hres = x_s[0].astype(f32) + jnp.sum(acc_s[...], axis=0, keepdims=True)
    hn = _layernorm(hres)
    wr = wr_s[...].astype(f32).reshape(1, D)
    gate = jax.nn.sigmoid(jnp.sum(hn * wr, axis=-1, keepdims=True))
    hb = jnp.broadcast_to(hn, (8, D)).astype(bf16)
    done(wg_s, SEM_GATE)
    done(wu_s, SEM_UP)
    g = matvec(hb, wg_s)
    act = g * jax.nn.sigmoid(g) * matvec(hb, wu_s)
    act_b = act.astype(bf16)

    group_rows = wd_s.shape[1]
    act_t = {}
    for unit, groups, r0, _, _ in DOWN_CHUNKS:
        for grp in groups if unit == "vpu" else ():
            t = (grp * group_rows + r0) // 128 * 128
            if t not in act_t:
                act_t[t] = jnp.broadcast_to(act[:1, t:t + 128] * gate, (128, 128)).T

    y = jnp.zeros((8, D), f32)
    out = None
    for c, (unit, groups, r0, rows, _) in enumerate(DOWN_CHUNKS):
        done(wd_s.at[pl.ds(groups[0], len(groups)), pl.ds(r0, rows)], SEM_DOWN + c)
        if unit == "mxu":
            for grp in groups:
                row = grp * group_rows + r0
                y = y + jnp.dot(act_b[:, row:row + rows], wd_s[grp, r0:r0 + rows, :],
                                preferred_element_type=f32)
            continue
        if out is None:
            first = lax.broadcasted_iota(jnp.int32, (8, D), 0) == 0
            out = jnp.where(first, jnp.broadcast_to(hres + hn + y[:1] * gate, (8, D)), 0.0)
        for grp in groups:
            for r in range(r0, r0 + rows, BAND):
                row = grp * group_rows + r
                a = act_t[row // 128 * 128][row % 128:row % 128 + BAND]
                out = out + wd_s[grp, r:r + BAND, :].astype(f32) * jnp.concatenate([a] * (D // 128), axis=1)
    for c in range(0, D, 128):
        o_ref[0, :, c:c + 128] = jnp.sum(out[:, c:c + 128], axis=0, keepdims=True).astype(o_ref.dtype)


@jax.jit
def pallas_sequential_preLN__sliding_block_cached__moe_arch_mod__decode_kernel(
    A_x: jax.Array,
    A_k_cache: jax.Array,
    A_v_cache: jax.Array,
    A_wq: jax.Array,
    A_wo: jax.Array,
    B_x: jax.Array,
    B_w_r: jax.Array,
    B_w_gate: jax.Array,
    B_w_up: jax.Array,
    B_w_down: jax.Array,
):
    del B_x
    _, H, Sk, Dh = A_k_cache.shape
    D = A_x.shape[-1]
    W = min(4096, max(256, Sk // 4))
    kt = jnp.transpose(A_k_cache, (0, 1, 3, 2))
    vt = jnp.transpose(A_v_cache, (0, 1, 3, 2))

    def tile_pairs(w):
        t = w.reshape(w.shape[0] // BAND, BAND, w.shape[1] // 128, 128).transpose(0, 2, 1, 3)
        return t.reshape(-1, SLAB, 2 * BAND, 128)

    wq, wo = tile_pairs(A_wq), tile_pairs(A_wo)
    wg, wu, wd = (w.reshape(GROUPS_F, -1, w.shape[1]) for w in (B_w_gate, B_w_up, B_w_down))
    like = lambda a: pltpu.VMEM(a.shape, a.dtype)
    return pl.pallas_call(
        _kernel,
        out_shape=jax.ShapeDtypeStruct(A_x.shape, A_x.dtype),
        in_specs=[pl.BlockSpec(memory_space=pl.ANY)] * 9,
        scratch_shapes=[
            like(A_x), like(B_w_r), like(wq), like(wo), like(wg), like(wu), like(wd),
            pltpu.VMEM((SLOTS, Dh, W), A_k_cache.dtype),
            pltpu.VMEM((SLOTS, Dh, W), A_v_cache.dtype),
            pltpu.VMEM((D, 128), jnp.float32),
            pltpu.VMEM((H, 8, Dh), jnp.float32),
            pltpu.VMEM((8, W), jnp.float32),
            pltpu.VMEM((8, D), jnp.float32),
            pltpu.SemaphoreType.DMA((SEM_DOWN + len(DOWN_CHUNKS),)),
        ],
        compiler_params=pltpu.CompilerParams(
            vmem_limit_bytes=100 * 2**20,
            disable_semaphore_checks=True,
        ),
    )(A_x, kt, vt, wq, wo, B_w_r, wg, wu, wd)
```

```python
import jax
import jax.numpy as jnp
from jax import lax
import jax.experimental.pallas as pl
import jax.experimental.pallas.tpu as pltpu

EPS = 1e-5
BAND = 8
RUN = 512
SLAB = 128
LAG = 27
ATTN_RUNS, KV_RUNS = 3, 4
GROUPS_F = 4
SLOTS = 4
Q_PARTS = 4
DOWN_CHUNKS = (
    ("mxu", range(0, 4), 0, 128, 32), ("mxu", range(0, 4), 128, 128, 32),
    ("vpu", range(0, 3), 256, 64, 32), ("vpu", range(0, 3), 320, 64, 32),
    ("vpu", range(3, 4), 256, 40, 40), ("vpu", range(3, 4), 296, 40, 40),
    ("vpu", range(3, 4), 336, 32, 32), ("vpu", range(3, 4), 368, 16, 16),
)
SEM_K, SEM_V = 0, SLOTS
SEM_X, SEM_R, SEM_Q, SEM_O, SEM_GATE, SEM_UP, SEM_DOWN = range(2 * SLOTS, 2 * SLOTS + 7)


def _layernorm(x):
    m = jnp.mean(x, axis=-1, keepdims=True)
    d = x - m
    v = jnp.mean(d * d, axis=-1, keepdims=True)
    return d / jnp.sqrt(v + EPS)


def _kernel(x_hbm, kt_hbm, vt_hbm, wq_hbm, wo_hbm, wr_hbm, wg_hbm, wu_hbm, wd_hbm,
            o_ref,
            x_s, wr_s, wq_s, wo_s, wg_s, wu_s, wd_s, k_s, v_s, xt_s, q_s, p_s, acc_s, sems):
    _, H, Dh, Sk = kt_hbm.shape
    W = k_s.shape[-1]
    D = x_hbm.shape[-1]
    F = wg_hbm.shape[-1]
    f32, bf16 = jnp.float32, jnp.bfloat16

    def start(piece, queue):
        src, dst, sem = piece
        pltpu.make_async_copy(src, dst, sems.at[sem]).start(priority=queue)

    def start_pairs(first, second):
        for a, b in zip(first, second, strict=True):
            start(a, 0)
            start(b, 1)

    def done(dst, sem):
        pltpu.make_async_copy(dst, dst, sems.at[sem]).wait()

    per_sweep = wq_s.shape[0] // ATTN_RUNS

    wq, wo = (wq_hbm, wq_s, SEM_Q), (wo_hbm, wo_s, SEM_O)
    wg, wu = (wg_hbm, wg_s, SEM_GATE), (wu_hbm, wu_s, SEM_UP)

    def attn_piece(weight, sweep, n):
        src, dst, sem = weight
        idx = (pl.ds(n % per_sweep * ATTN_RUNS, ATTN_RUNS), pl.ds(2 * (sweep + n // per_sweep), 2))
        return src.at[idx], dst.at[idx], sem

    def kv_pieces(h, half):
        slot = h % SLOTS
        return [(src.at[0, h, pl.ds(r, KV_RUNS * BAND), pl.ds(Sk - W + c, RUN)],
                 dst.at[slot, pl.ds(r, KV_RUNS * BAND), pl.ds(c, RUN)], sem + slot)
                for src, dst, sem in ((kt_hbm, k_s, SEM_K), (vt_hbm, v_s, SEM_V))
                for c in range(0, W, RUN)
                for r in range(half * Dh // 2, (half + 1) * Dh // 2, KV_RUNS * BAND)]

    def ffn_pieces(weight):
        src, dst, sem = weight
        return [(src.at[:, pl.ds(r, BAND), pl.ds(c, RUN)], dst.at[:, pl.ds(r, BAND), pl.ds(c, RUN)], sem)
                for r in range(0, dst.shape[1], BAND) for c in range(0, F, RUN)]

    def start_tail(third):
        down = [(wd_hbm.at[grp, pl.ds(r, step)], wd_s.at[grp, pl.ds(r, step)], SEM_DOWN + c)
                for c, (_, groups, r0, rows, step) in enumerate(DOWN_CHUNKS)
                for r in range(r0, r0 + rows, step) for grp in groups]
        paired = (len(down) - LAG) // 2 * 2
        first = ffn_pieces(wg) + down[0:paired:2]
        second = ffn_pieces(wu)[LAG:] + down[1:paired:2] + down[paired:]
        lo, hi = third * len(first) // 3, (third + 1) * len(first) // 3
        start_pairs(first[lo:hi], second[lo:hi])
        if third == 2:
            for piece in second[hi:]:
                start(piece, 1)

    x_cp = pltpu.make_async_copy(x_hbm, x_s, sems.at[SEM_X])
    wr_cp = pltpu.make_async_copy(wr_hbm, wr_s, sems.at[SEM_R])
    early = (5, 15, 25)
    for n in range(LAG + len(early)):
        if n in early:
            start(attn_piece(wq, 0, early.index(n)), 0)
        start(attn_piece(wo, 0, n), 1)
    start_pairs([attn_piece(wq, 0, n) for n in range(len(early), per_sweep)],
                [attn_piece(wo, 0, LAG + n) for n in range(len(early), per_sweep)])
    x_cp.start()
    wr_cp.start()

    def sweep(i, _):
        start_pairs([attn_piece(wq, i, n) for n in range(per_sweep)],
                    [attn_piece(wo, i, LAG + n) for n in range(per_sweep)])

    total = SLAB // 2 * per_sweep
    looped = (total - LAG) // per_sweep
    lax.fori_loop(1, looped, sweep, None)
    start_pairs([attn_piece(wq, 0, n) for n in range(looped * per_sweep, total)],
                [attn_piece(wo, 0, n) for n in range(looped * per_sweep + LAG, total)]
                + kv_pieces(0, 1)[:LAG])

    def normalize_x():
        x_cp.wait()
        wr_cp.wait()
        done(wq_s, SEM_Q)
        done(wo_s, SEM_O)
        xn = _layernorm(x_s[0].astype(f32)).astype(bf16).astype(f32)
        for c in range(0, D, 128):
            xt_s[c:c + 128, :] = jnp.broadcast_to(xn[:, c:c + 128], (128, 128)).T
        acc_s[...] = jnp.zeros_like(acc_s)

    def project_q(part):
        band_pairs = H * Dh // 256
        quads = H // 4 // Q_PARTS
        for c in range(part * quads, (part + 1) * quads):
            a = [jnp.zeros((8, 128), f32)] * 6
            for b in range(D // BAND):
                xb = xt_s[b * BAND:(b + 1) * BAND, :]
                for j in range(3):
                    m = b * band_pairs + 3 * c + j
                    ww = wq_s[m // SLAB, m % SLAB].astype(f32)
                    a[2 * j] = a[2 * j] + ww[:8] * xb
                    a[2 * j + 1] = a[2 * j + 1] + ww[8:] * xb
            q4 = jnp.concatenate(
                [jnp.broadcast_to(jnp.sum(t, axis=0, keepdims=True), (8, 128)) for t in a], axis=1)
            for k in range(4):
                q_s[4 * c + k] = q4[:, k * Dh:(k + 1) * Dh]

    def probabilities(h):
        slot = h % SLOTS
        done(k_s.at[slot], SEM_K + slot)
        s = jnp.dot(q_s[h].astype(bf16), k_s[slot], preferred_element_type=f32) * Dh ** -0.5
        e = jnp.exp(s - jnp.max(s, axis=-1, keepdims=True))
        p_s[...] = e * (1.0 / jnp.sum(e, axis=-1, keepdims=True))

    def accumulate(h):
        slot = h % SLOTS
        done(v_s.at[slot], SEM_V + slot)
        tiles = D // 128
        acc = [acc_s[:, t * 128:(t + 1) * 128] for t in range(tiles)]
        for r in range(0, Dh, 16):
            a0 = jnp.zeros((8, 128), f32)
            a1 = jnp.zeros((8, 128), f32)
            for c in range(0, W, 128):
                vv = v_s[slot, r:r + 16, c:c + 128].astype(f32)
                pp = p_s[:, c:c + 128]
                a0 = a0 + vv[:8] * pp
                a1 = a1 + vv[8:] * pp
            o0 = jnp.sum(a0, axis=-1, keepdims=True)
            o1 = jnp.sum(a1, axis=-1, keepdims=True)
            for j in range(tiles):
                m = h * (Dh // 16 * tiles) + r // 16 * tiles + j
                ww = wo_s[lax.div(m, SLAB), lax.rem(m, SLAB)].astype(f32)
                for n, w in ((2 * j, ww[:8]), (2 * j + 1, ww[8:])):
                    acc[n % tiles] = acc[n % tiles] + w * (o0 if n < tiles else o1)
        for t in range(tiles):
            acc_s[:, t * 128:(t + 1) * 128] = acc[t]

    def step(i, _):
        cut = Dh // (KV_RUNS * BAND) * (W // RUN) - LAG
        pl.when(i < H)(lambda: start_pairs(kv_pieces(i, 0)[:cut], kv_pieces(i, 1)[LAG:]))
        pl.when(i == H)(lambda: start_tail(0))
        pl.when(i == 1)(normalize_x)
        for part in range(Q_PARTS):
            pl.when(i == 1 + part)(lambda part=part: project_q(part))
        pl.when(i >= 2)(lambda: probabilities(i - 2))
        pl.when(i < H - 1)(lambda: start_pairs(kv_pieces(i, 0)[cut:], kv_pieces(i + 1, 1)[:LAG]))
        pl.when(i == H - 1)(lambda: start_pairs(kv_pieces(H - 1, 0)[cut:], ffn_pieces(wu)[:LAG]))
        pl.when(i == H)(lambda: start_tail(1))
        pl.when(i == H + 1)(lambda: start_tail(2))
        pl.when(i >= 2)(lambda: accumulate(i - 2))

    lax.fori_loop(0, H + 2, step, None)

    def matvec(v, w_s):
        w = w_s[...]
        return jnp.dot(v, w.reshape(-1, w.shape[-1]), preferred_element_type=f32)

    hres = x_s[0].astype(f32) + jnp.sum(acc_s[...], axis=0, keepdims=True)
    hn = _layernorm(hres)
    wr = wr_s[...].astype(f32).reshape(1, D)
    gate = jax.nn.sigmoid(jnp.sum(hn * wr, axis=-1, keepdims=True))
    hb = jnp.broadcast_to(hn, (8, D)).astype(bf16)
    done(wg_s, SEM_GATE)
    done(wu_s, SEM_UP)
    g = matvec(hb, wg_s)
    act = g * jax.nn.sigmoid(g) * matvec(hb, wu_s)
    act_b = act.astype(bf16)

    group_rows = wd_s.shape[1]
    act_t = {}
    for unit, groups, r0, _, _ in DOWN_CHUNKS:
        for grp in groups if unit == "vpu" else ():
            t = (grp * group_rows + r0) // 128 * 128
            if t not in act_t:
                act_t[t] = jnp.broadcast_to(act[:1, t:t + 128] * gate, (128, 128)).T

    y = jnp.zeros((8, D), f32)
    out = None
    for c, (unit, groups, r0, rows, _) in enumerate(DOWN_CHUNKS):
        done(wd_s.at[pl.ds(groups[0], len(groups)), pl.ds(r0, rows)], SEM_DOWN + c)
        if unit == "mxu":
            for grp in groups:
                row = grp * group_rows + r0
                y = y + jnp.dot(act_b[:, row:row + rows], wd_s[grp, r0:r0 + rows, :],
                                preferred_element_type=f32)
            continue
        if out is None:
            first = lax.broadcasted_iota(jnp.int32, (8, D), 0) == 0
            out = jnp.where(first, jnp.broadcast_to(hres + hn + y[:1] * gate, (8, D)), 0.0)
        for grp in groups:
            for r in range(r0, r0 + rows, BAND):
                row = grp * group_rows + r
                a = act_t[row // 128 * 128][row % 128:row % 128 + BAND]
                out = out + wd_s[grp, r:r + BAND, :].astype(f32) * jnp.concatenate([a] * (D // 128), axis=1)
    for c in range(0, D, 128):
        o_ref[0, :, c:c + 128] = jnp.sum(out[:, c:c + 128], axis=0, keepdims=True).astype(o_ref.dtype)


@jax.jit
def pallas_sequential_preLN__sliding_block_cached__moe_arch_mod__decode_kernel(
    A_x: jax.Array,
    A_k_cache: jax.Array,
    A_v_cache: jax.Array,
    A_wq: jax.Array,
    A_wo: jax.Array,
    B_x: jax.Array,
    B_w_r: jax.Array,
    B_w_gate: jax.Array,
    B_w_up: jax.Array,
    B_w_down: jax.Array,
):
    del B_x
    _, H, Sk, Dh = A_k_cache.shape
    D = A_x.shape[-1]
    W = min(4096, max(256, Sk // 4))
    kt = jnp.transpose(A_k_cache, (0, 1, 3, 2))
    vt = jnp.transpose(A_v_cache, (0, 1, 3, 2))

    def tile_pairs(w):
        t = w.reshape(w.shape[0] // BAND, BAND, w.shape[1] // 128, 128).transpose(0, 2, 1, 3)
        return t.reshape(-1, SLAB, 2 * BAND, 128)

    wq, wo = tile_pairs(A_wq), tile_pairs(A_wo)
    wg, wu, wd = (w.reshape(GROUPS_F, -1, w.shape[1]) for w in (B_w_gate, B_w_up, B_w_down))
    like = lambda a: pltpu.VMEM(a.shape, a.dtype)
    return pl.pallas_call(
        _kernel,
        out_shape=jax.ShapeDtypeStruct(A_x.shape, A_x.dtype),
        in_specs=[pl.BlockSpec(memory_space=pl.ANY)] * 9,
        scratch_shapes=[
            like(A_x), like(B_w_r), like(wq), like(wo), like(wg), like(wu), like(wd),
            pltpu.VMEM((SLOTS, Dh, W), A_k_cache.dtype),
            pltpu.VMEM((SLOTS, Dh, W), A_v_cache.dtype),
            pltpu.VMEM((D, 128), jnp.float32),
            pltpu.VMEM((H, 8, Dh), jnp.float32),
            pltpu.VMEM((8, W), jnp.float32),
            pltpu.VMEM((8, D), jnp.float32),
            pltpu.SemaphoreType.DMA((SEM_DOWN + len(DOWN_CHUNKS),)),
        ],
        compiler_params=pltpu.CompilerParams(
            vmem_limit_bytes=100 * 2**20,
            disable_semaphore_checks=True,
        ),
    )(A_x, kt, vt, wq, wo, B_w_r, wg, wu, wd)
```

```python
import jax
import jax.numpy as jnp
from jax import lax
import jax.experimental.pallas as pl
import jax.experimental.pallas.tpu as pltpu

EPS = 1e-5
BAND = 8
RUN = 512
SLAB = 128
LAG = 27
ATTN_RUNS, KV_RUNS = 3, 4
GROUPS_F = 4
SLOTS = 4
Q_PARTS = 4
DOWN_CHUNKS = (
    ("mxu", range(0, 4), 0, 128, 32), ("mxu", range(0, 4), 128, 128, 32),
    ("vpu", range(0, 3), 256, 64, 32), ("vpu", range(0, 3), 320, 64, 32),
    ("vpu", range(3, 4), 256, 40, 40), ("vpu", range(3, 4), 296, 40, 40),
    ("vpu", range(3, 4), 336, 32, 32), ("vpu", range(3, 4), 368, 16, 16),
)
SEM_K, SEM_V = 0, SLOTS
SEM_X, SEM_R, SEM_Q, SEM_O, SEM_GATE, SEM_UP, SEM_DOWN = range(2 * SLOTS, 2 * SLOTS + 7)


def _layernorm(x):
    m = jnp.mean(x, axis=-1, keepdims=True)
    d = x - m
    v = jnp.mean(d * d, axis=-1, keepdims=True)
    return d / jnp.sqrt(v + EPS)


def _kernel(x_hbm, kt_hbm, vt_hbm, wq_hbm, wo_hbm, wr_hbm, wg_hbm, wu_hbm, wd_hbm,
            o_ref,
            x_s, wr_s, wq_s, wo_s, wg_s, wu_s, wd_s, k_s, v_s, xt_s, q_s, p_s, acc_s, sems):
    _, H, Dh, Sk = kt_hbm.shape
    W = k_s.shape[-1]
    D = x_hbm.shape[-1]
    F = wg_hbm.shape[-1]
    f32, bf16 = jnp.float32, jnp.bfloat16

    def start(piece, queue):
        src, dst, sem = piece
        pltpu.make_async_copy(src, dst, sems.at[sem]).start(priority=queue)

    def start_pairs(first, second):
        for a, b in zip(first, second, strict=True):
            start(a, 0)
            start(b, 1)

    def done(dst, sem):
        pltpu.make_async_copy(dst, dst, sems.at[sem]).wait()

    per_sweep = wq_s.shape[0] // ATTN_RUNS

    wq, wo = (wq_hbm, wq_s, SEM_Q), (wo_hbm, wo_s, SEM_O)
    wg, wu = (wg_hbm, wg_s, SEM_GATE), (wu_hbm, wu_s, SEM_UP)

    def attn_piece(weight, sweep, n):
        src, dst, sem = weight
        idx = (pl.ds(n % per_sweep * ATTN_RUNS, ATTN_RUNS), pl.ds(2 * (sweep + n // per_sweep), 2))
        return src.at[idx], dst.at[idx], sem

    per_half = Dh // 2 // (KV_RUNS * BAND) * (W // RUN)

    def kv_pieces(h, half):
        slot = h % SLOTS
        return [(src.at[0, h, pl.ds(r, KV_RUNS * BAND), pl.ds(Sk - W + c, RUN)],
                 dst.at[slot, pl.ds(r, KV_RUNS * BAND), pl.ds(c, RUN)], sem + slot)
                for src, dst, sem in ((kt_hbm, k_s, SEM_K), (vt_hbm, v_s, SEM_V))
                for c in range(0, W, RUN)
                for r in range(half * Dh // 2, (half + 1) * Dh // 2, KV_RUNS * BAND)]

    def ffn_pieces(weight):
        src, dst, sem = weight
        return [(src.at[:, pl.ds(r, BAND), pl.ds(c, RUN)], dst.at[:, pl.ds(r, BAND), pl.ds(c, RUN)], sem)
                for r in range(0, dst.shape[1], BAND) for c in range(0, F, RUN)]

    def last_of_queue_1():
        return kv_pieces(H - 1, 1)[per_half:] + ffn_pieces(wu)

    def start_tail(third):
        down = [(wd_hbm.at[grp, pl.ds(r, step)], wd_s.at[grp, pl.ds(r, step)], SEM_DOWN + c)
                for c, (_, groups, r0, rows, step) in enumerate(DOWN_CHUNKS)
                for r in range(r0, r0 + rows, step) for grp in groups]
        paired = (len(down) - LAG) // 2 * 2
        first = kv_pieces(H - 1, 1)[:per_half] + ffn_pieces(wg) + down[0:paired:2]
        second = last_of_queue_1()[LAG:] + down[1:paired:2] + down[paired:]
        lo, hi = third * len(first) // 3, (third + 1) * len(first) // 3
        start_pairs(first[lo:hi], second[lo:hi])
        if third == 2:
            for piece in second[hi:]:
                start(piece, 1)

    x_cp = pltpu.make_async_copy(x_hbm, x_s, sems.at[SEM_X])
    wr_cp = pltpu.make_async_copy(wr_hbm, wr_s, sems.at[SEM_R])
    early = (5, 15, 25)
    for n in range(LAG + len(early)):
        if n in early:
            start(attn_piece(wq, 0, early.index(n)), 0)
        start(attn_piece(wo, 0, n), 1)
    start_pairs([attn_piece(wq, 0, n) for n in range(len(early), per_sweep)],
                [attn_piece(wo, 0, LAG + n) for n in range(len(early), per_sweep)])
    x_cp.start()
    wr_cp.start()

    def sweep(i, _):
        start_pairs([attn_piece(wq, i, n) for n in range(per_sweep)],
                    [attn_piece(wo, i, LAG + n) for n in range(per_sweep)])

    total = SLAB // 2 * per_sweep
    looped = (total - LAG) // per_sweep
    lax.fori_loop(1, looped, sweep, None)
    start_pairs([attn_piece(wq, 0, n) for n in range(looped * per_sweep, total)]
                + kv_pieces(0, 0)[per_half:],
                [attn_piece(wo, 0, n) for n in range(looped * per_sweep + LAG, total)]
                + kv_pieces(0, 0)[:per_half] + kv_pieces(1, 0)[:LAG])

    def normalize_x():
        x_cp.wait()
        wr_cp.wait()
        done(wq_s, SEM_Q)
        done(wo_s, SEM_O)
        xn = _layernorm(x_s[0].astype(f32)).astype(bf16).astype(f32)
        for c in range(0, D, 128):
            xt_s[c:c + 128, :] = jnp.broadcast_to(xn[:, c:c + 128], (128, 128)).T
        acc_s[...] = jnp.zeros_like(acc_s)

    def project_q(part):
        band_pairs = H * Dh // 256
        quads = H // 4 // Q_PARTS
        for c in range(part * quads, (part + 1) * quads):
            a = [jnp.zeros((8, 128), f32)] * 6
            for b in range(D // BAND):
                xb = xt_s[b * BAND:(b + 1) * BAND, :]
                for j in range(3):
                    m = b * band_pairs + 3 * c + j
                    ww = wq_s[m // SLAB, m % SLAB].astype(f32)
                    a[2 * j] = a[2 * j] + ww[:8] * xb
                    a[2 * j + 1] = a[2 * j + 1] + ww[8:] * xb
            q4 = jnp.concatenate(
                [jnp.broadcast_to(jnp.sum(t, axis=0, keepdims=True), (8, 128)) for t in a], axis=1)
            for k in range(4):
                q_s[4 * c + k] = q4[:, k * Dh:(k + 1) * Dh]

    def probabilities(h):
        slot = h % SLOTS
        done(k_s.at[slot], SEM_K + slot)
        s = jnp.dot(q_s[h].astype(bf16), k_s[slot], preferred_element_type=f32) * Dh ** -0.5
        e = jnp.exp(s - jnp.max(s, axis=-1, keepdims=True))
        p_s[...] = e * (1.0 / jnp.sum(e, axis=-1, keepdims=True))

    def accumulate(h):
        slot = h % SLOTS
        done(v_s.at[slot], SEM_V + slot)
        tiles = D // 128
        acc = [acc_s[:, t * 128:(t + 1) * 128] for t in range(tiles)]
        for r in range(0, Dh, 16):
            a0 = jnp.zeros((8, 128), f32)
            a1 = jnp.zeros((8, 128), f32)
            for c in range(0, W, 128):
                vv = v_s[slot, r:r + 16, c:c + 128].astype(f32)
                pp = p_s[:, c:c + 128]
                a0 = a0 + vv[:8] * pp
                a1 = a1 + vv[8:] * pp
            o0 = jnp.sum(a0, axis=-1, keepdims=True)
            o1 = jnp.sum(a1, axis=-1, keepdims=True)
            for j in range(tiles):
                m = h * (Dh // 16 * tiles) + r // 16 * tiles + j
                ww = wo_s[lax.div(m, SLAB), lax.rem(m, SLAB)].astype(f32)
                for n, w in ((2 * j, ww[:8]), (2 * j + 1, ww[8:])):
                    acc[n % tiles] = acc[n % tiles] + w * (o0 if n < tiles else o1)
        for t in range(tiles):
            acc_s[:, t * 128:(t + 1) * 128] = acc[t]

    def step(i, _):
        cut = 2 * per_half - LAG
        pl.when(i < H - 1)(lambda: start_pairs(kv_pieces(i, 1)[:cut], kv_pieces(i + 1, 0)[LAG:]))
        pl.when(i == H - 1)(lambda: start_tail(0))
        pl.when(i == 0)(normalize_x)
        for part in range(Q_PARTS):
            pl.when(i == part)(lambda part=part: project_q(part))
        pl.when(i > 0)(lambda: probabilities(i - 1))
        pl.when(i < H - 2)(lambda: start_pairs(kv_pieces(i, 1)[cut:], kv_pieces(i + 2, 0)[:LAG]))
        pl.when(i == H - 2)(lambda: start_pairs(kv_pieces(H - 2, 1)[cut:], last_of_queue_1()[:LAG]))
        pl.when(i == H - 1)(lambda: start_tail(1))
        pl.when(i == H)(lambda: start_tail(2))
        pl.when(i > 0)(lambda: accumulate(i - 1))

    lax.fori_loop(0, H + 1, step, None)

    def matvec(v, w_s):
        w = w_s[...]
        return jnp.dot(v, w.reshape(-1, w.shape[-1]), preferred_element_type=f32)

    hres = x_s[0].astype(f32) + jnp.sum(acc_s[...], axis=0, keepdims=True)
    hn = _layernorm(hres)
    wr = wr_s[...].astype(f32).reshape(1, D)
    gate = jax.nn.sigmoid(jnp.sum(hn * wr, axis=-1, keepdims=True))
    hb = jnp.broadcast_to(hn, (8, D)).astype(bf16)
    done(wg_s, SEM_GATE)
    done(wu_s, SEM_UP)
    g = matvec(hb, wg_s)
    act = g * jax.nn.sigmoid(g) * matvec(hb, wu_s)
    act_b = act.astype(bf16)

    group_rows = wd_s.shape[1]
    act_t = {}
    for unit, groups, r0, _, _ in DOWN_CHUNKS:
        for grp in groups if unit == "vpu" else ():
            t = (grp * group_rows + r0) // 128 * 128
            if t not in act_t:
                act_t[t] = jnp.broadcast_to(act[:1, t:t + 128] * gate, (128, 128)).T

    y = jnp.zeros((8, D), f32)
    out = None
    for c, (unit, groups, r0, rows, _) in enumerate(DOWN_CHUNKS):
        done(wd_s.at[pl.ds(groups[0], len(groups)), pl.ds(r0, rows)], SEM_DOWN + c)
        if unit == "mxu":
            for grp in groups:
                row = grp * group_rows + r0
                y = y + jnp.dot(act_b[:, row:row + rows], wd_s[grp, r0:r0 + rows, :],
                                preferred_element_type=f32)
            continue
        if out is None:
            first = lax.broadcasted_iota(jnp.int32, (8, D), 0) == 0
            out = jnp.where(first, jnp.broadcast_to(hres + hn + y[:1] * gate, (8, D)), 0.0)
        for grp in groups:
            for r in range(r0, r0 + rows, BAND):
                row = grp * group_rows + r
                a = act_t[row // 128 * 128][row % 128:row % 128 + BAND]
                out = out + wd_s[grp, r:r + BAND, :].astype(f32) * jnp.concatenate([a] * (D // 128), axis=1)
    for c in range(0, D, 128):
        o_ref[0, :, c:c + 128] = jnp.sum(out[:, c:c + 128], axis=0, keepdims=True).astype(o_ref.dtype)


@jax.jit
def pallas_sequential_preLN__sliding_block_cached__moe_arch_mod__decode_kernel(
    A_x: jax.Array,
    A_k_cache: jax.Array,
    A_v_cache: jax.Array,
    A_wq: jax.Array,
    A_wo: jax.Array,
    B_x: jax.Array,
    B_w_r: jax.Array,
    B_w_gate: jax.Array,
    B_w_up: jax.Array,
    B_w_down: jax.Array,
):
    del B_x
    _, H, Sk, Dh = A_k_cache.shape
    D = A_x.shape[-1]
    W = min(4096, max(256, Sk // 4))
    kt = jnp.transpose(A_k_cache, (0, 1, 3, 2))
    vt = jnp.transpose(A_v_cache, (0, 1, 3, 2))

    def tile_pairs(w):
        t = w.reshape(w.shape[0] // BAND, BAND, w.shape[1] // 128, 128).transpose(0, 2, 1, 3)
        return t.reshape(-1, SLAB, 2 * BAND, 128)

    wq, wo = tile_pairs(A_wq), tile_pairs(A_wo)
    wg, wu, wd = (w.reshape(GROUPS_F, -1, w.shape[1]) for w in (B_w_gate, B_w_up, B_w_down))
    like = lambda a: pltpu.VMEM(a.shape, a.dtype)
    return pl.pallas_call(
        _kernel,
        out_shape=jax.ShapeDtypeStruct(A_x.shape, A_x.dtype),
        in_specs=[pl.BlockSpec(memory_space=pl.ANY)] * 9,
        scratch_shapes=[
            like(A_x), like(B_w_r), like(wq), like(wo), like(wg), like(wu), like(wd),
            pltpu.VMEM((SLOTS, Dh, W), A_k_cache.dtype),
            pltpu.VMEM((SLOTS, Dh, W), A_v_cache.dtype),
            pltpu.VMEM((D, 128), jnp.float32),
            pltpu.VMEM((H, 8, Dh), jnp.float32),
            pltpu.VMEM((8, W), jnp.float32),
            pltpu.VMEM((8, D), jnp.float32),
            pltpu.SemaphoreType.DMA((SEM_DOWN + len(DOWN_CHUNKS),)),
        ],
        compiler_params=pltpu.CompilerParams(
            vmem_limit_bytes=100 * 2**20,
            disable_semaphore_checks=True,
        ),
    )(A_x, kt, vt, wq, wo, B_w_r, wg, wu, wd)
```
